```python
import os as _os
_os.environ.setdefault("JAX_PLATFORMS", "cpu")
import jax
import jax.numpy as jnp

def _softmax(x, axis=-1):
    return jax.nn.softmax(x, axis=axis)
def _gelu(x):
    return jax.nn.gelu(x, approximate=True)
def _silu(x):
    return jax.nn.silu(x)
def _sigmoid(x):
    return jax.nn.sigmoid(x)
def _layernorm(x, axis=-1, eps=1e-5):
    m = jnp.mean(x, axis=axis, keepdims=True)
    v = jnp.var(x, axis=axis, keepdims=True)
    return (x - m) / jnp.sqrt(v + eps)
def _scatter_add(tgt, idx, src, axis=0):
    return tgt.at[idx].add(src)
def _segment_sum(src, seg, n):
    return jax.ops.segment_sum(src, seg, n)
class _Rng:
    def __init__(self, key):
        self._k = key
    def _next(self):
        self._k, sub = jax.random.split(self._k)
        return sub
    def normal(self, shape):
        return jax.random.normal(self._next(), shape, dtype=jnp.bfloat16)
    def randint(self, lo, hi, shape):
        return jax.random.randint(self._next(), shape, lo, hi, dtype=jnp.int32)
    def uniform(self, shape, lo=0.0, hi=1.0):
        return jax.random.uniform(self._next(), shape, jnp.bfloat16, lo, hi)
    def permutation(self, n):
        return jax.random.permutation(self._next(), n)


kernel_name = 'sequential_preLN__mha_block__mixer_token_mlp__prompt'

def setup_inputs():
    _rng = _Rng(jax.random.key(int.from_bytes(__import__("os").urandom(4), "little")))
    _w = (lambda a: (lambda t: t.astype(jnp.bfloat16) if jnp.issubdtype(t.dtype, jnp.floating) else t)(jnp.asarray(a)))
    def _A_setup():
        B, S, D, H = 1, 2048, 448, 16
        return {
            "x": _w((lambda *s: _rng.normal(s) * 0.05)(B, S, D)),
            "wqkv": _w((lambda *s: _rng.normal(s) * 0.05)(D, 3 * D)),
            "wo": _w((lambda *s: _rng.normal(s) * 0.05)(D, D)),
        }
    _A_in = _A_setup()

    def _B_setup():
        B, S, D, F = 1, 2048, 448, 1792
        return {
            "x": _w((lambda *s: _rng.normal(s) * 0.05)(B, S, D)),
            "w1": _w((lambda *s: _rng.normal(s) * 0.2)(S, F) * (S ** -0.5)),
            "b1": _w((lambda *s: _rng.normal(s) * 0.2)(F) * 0.02),
            "w2": _w((lambda *s: _rng.normal(s) * 0.2)(F, S) * (F ** -0.5)),
            "b2": _w((lambda *s: _rng.normal(s) * 0.05)(S) * 0.02),
        }
    _B_in = _B_setup()

    return {
        "A_x": _A_in["x"],
        "A_wqkv": _A_in["wqkv"],
        "A_wo": _A_in["wo"],
        "B_x": _B_in["x"],
        "B_w1": _B_in["w1"],
        "B_b1": _B_in["b1"],
        "B_w2": _B_in["w2"],
        "B_b2": _B_in["b2"],
    }

def reference(A_x, A_wqkv, A_wo, B_x, B_w1, B_b1, B_w2, B_b2):
    def _A_ref(x, wqkv, wo):
        B, S, D = x.shape
        H = 16
        Dh = D // H
        qkv = (lambda x, *d: x.transpose(*d))((x @ wqkv).reshape(B, S, 3, H, Dh), 2, 0, 3, 1, 4)
        q, k, v = qkv[0], qkv[1], qkv[2]
        scores = jnp.einsum("bhqd,bhkd->bhqk", q, k) * (Dh ** -0.5)
        p = _softmax(scores, axis=-1)
        o = jnp.einsum("bhqk,bhkd->bhqd", p, v)
        return (lambda x, *d: x.transpose(*d))(o, 0, 2, 1, 3).reshape(B, S, D) @ wo

    def _B_ref(x, w1, b1, w2, b2):
        B, S, D = x.shape
        h = _layernorm(x, axis=-1)
        u = jnp.einsum("bsd,sf->bdf", h, w1) + b1
        u = _gelu(u)
        y = jnp.einsum("bdf,fs->bds", u, w2) + b2
        return (lambda x, *d: x.transpose(*d))(y, 0, 2, 1)

    x = A_x
    h = x + _A_ref(_layernorm(x, axis=-1), A_wqkv, A_wo)
    h2 = h + _B_ref(_layernorm(h, axis=-1), B_w1, B_b1, B_w2, B_b2)
    return h2
```

```python
import functools
import math

import jax
import jax.numpy as jnp
import jax.experimental.pallas as pl
import jax.experimental.pallas.tpu as pltpu

S = 2048
D = 448
H = 16
DH = 28
F = 1792
HPG = 4
NG = H // HPG
GW = HPG * DH
HP = 32
EPS = 1e-5

TS1 = 512
TQ = 512
TK = 128
LOOKAHEAD = 2
UNITS = 8
TS3 = 512
TF4 = 256
TS5 = 256

NQ = S // TQ
NK = S // TK
NU = H * NQ
STEPS = UNITS * NK
RING = LOOKAHEAD + 1
while STEPS % RING:
    RING += 1

N1 = S // TS1
N5 = S // TS5

SEM_X = 0
SEM_WQKV = SEM_X + N1
SEM_WO = SEM_WQKV + 1
SEM_B1 = SEM_WO + 1
SEM_B2 = SEM_B1 + 1
SEM_W1 = SEM_B2 + 1
SEM_W2 = SEM_W1 + 1
SEM_OUT = SEM_W2 + 1
NSEM = SEM_OUT + N5

_NT = (((1,), (1,)), ((), ()))
_F32 = jnp.float32
_BF16 = jnp.bfloat16


def _dot(a, b):
    return jnp.dot(a, b, preferred_element_type=_F32)


def _dot_nt(a, b):
    return jax.lax.dot_general(a, b, _NT, preferred_element_type=_F32)


def _pad_head_rows(w):
    zeros = jnp.zeros((HP - DH, w.shape[1]), w.dtype)
    parts = []
    for h in range(H):
        parts.append(w[h * DH:(h + 1) * DH, :])
        parts.append(zeros)
    return jnp.concatenate(parts, axis=0)


def _kernel(x_hbm, wqkv_hbm, wo_hbm, w1_hbm, b1_hbm, w2_hbm, b2_hbm, out_hbm,
            x_v, wqkv_v, wo_v, w1_v, b1_v, w2_v, b2_v,
            wk_g, wqv_t, wo_t, k_v, qt_v, vt_v, ot_v, ht_v, hnt_v, g_v, out_v,
            sems, *ring):
    s_ring = ring[:RING]
    m_ring = ring[RING:]

    def copy(src, dst, sem):
        return pltpu.make_async_copy(src, dst, sems.at[sem])

    def x_copy(c):
        rows = pl.ds(c * TS1, TS1)
        return copy(x_hbm.at[rows, :], x_v.at[rows, :], SEM_X + c)

    def out_copy(c):
        rows = pl.ds(c * TS5, TS5)
        return copy(out_v.at[rows, :], out_hbm.at[rows, :], SEM_OUT + c)

    wqkv_copy = copy(wqkv_hbm, wqkv_v, SEM_WQKV)
    wo_copy = copy(wo_hbm, wo_v, SEM_WO)
    b1_copy = copy(b1_hbm, b1_v, SEM_B1)
    b2_copy = copy(b2_hbm, b2_v, SEM_B2)
    w1_copy = copy(w1_hbm, w1_v, SEM_W1)
    w2_copy = copy(w2_hbm, w2_v, SEM_W2)

    wqkv_copy.start()
    for c in range(N1):
        x_copy(c).start()
    wo_copy.start()
    b1_copy.start()
    b2_copy.start()

    wqkv_copy.wait()
    for g in range(NG):
        wk_g[g] = wqkv_v[:, D + g * GW:D + (g + 1) * GW]
    wqv_t[0:D, :] = wqkv_v[:, 0:D].T
    wv_t = wqkv_v[:, 2 * D:3 * D].astype(_F32).T
    wqv_t[D:, :] = _pad_head_rows(wv_t).astype(_BF16)

    q_scale = (DH ** -0.5) * math.log2(math.e)
    for c in range(N1):
        x_copy(c).wait()
        if c == N1 - 1:
            w1_copy.start()
            w2_copy.start()
        rows = slice(c * TS1, (c + 1) * TS1)
        xb = x_v[rows, :]
        xf = xb.astype(_F32)
        mu = jnp.mean(xf, axis=-1, keepdims=True)
        xc = xf - mu
        var = jnp.mean(xc * xc, axis=-1, keepdims=True)
        xn = (xc * jax.lax.rsqrt(var + EPS)).astype(_BF16)
        for g in range(NG):
            k_v[g, rows, :] = _dot(xn, wk_g[g]).astype(_BF16)
        qv = _dot_nt(wqv_t[...], xn)
        for g in range(NG):
            qt_v[g, :, rows] = (qv[g * GW:(g + 1) * GW, :] * q_scale).astype(_BF16)
        vt = qv[D:, :]
        rid = jax.lax.broadcasted_iota(jnp.int32, vt.shape, 0)
        vt = jnp.where(rid % HP == DH, 1.0, vt)
        vt_v[:, rows] = vt.astype(_BF16)
        ht_v[:, rows] = xf.T

    wo_copy.wait()
    wo_t[...] = _pad_head_rows(wo_v[...].astype(_F32)).astype(_BF16).T

    def get_wq(u):
        h = u // NQ
        qi = u % NQ
        g = h // HPG
        j = h % HPG
        qoff = pl.multiple_of(qi * TQ, TQ)
        wq = qt_v[g, :, pl.ds(qoff, TQ)]
        rid = jax.lax.broadcasted_iota(jnp.int32, (GW, TQ), 0)
        keep = (rid >= DH * j) & (rid < DH * j + DH)
        return jnp.where(keep, wq, jnp.zeros_like(wq)), g

    def score_chunk(slot, g, wq, kc, m_prev):
        s = _dot(k_v[g, kc * TK:(kc + 1) * TK, :], wq)
        s_ring[slot][...] = s
        cm = jnp.max(jnp.max(s.reshape(TK // 8, 8, TQ), axis=0), axis=0, keepdims=True)
        m = cm if m_prev is None else jnp.maximum(m_prev, cm)
        m_ring[slot][...] = m
        return m

    wq0, g0 = get_wq(0)
    m0 = None
    for t in range(LOOKAHEAD):
        m0 = score_chunk(t % RING, g0, wq0, t, m0)

    def attn_body(i, carry):
        u0 = i * UNITS
        wqs = {}
        ms = {}

        def wq_of(ul):
            if ul not in wqs:
                wqs[ul] = get_wq(jnp.minimum(u0 + ul, NU - 1))
            return wqs[ul]

        def m_of(t):
            if t not in ms:
                ms[t] = m_ring[t % RING][...]
            return ms[t]

        acc = None
        for t in range(STEPS):
            ta = t + LOOKAHEAD
            ul, kc = divmod(ta, NK)
            wq, g = wq_of(ul)
            ms[ta] = score_chunk(ta % RING, g, wq, kc, None if kc == 0 else m_of(ta - 1))
            ul, kc = divmod(t, NK)
            u = u0 + ul
            h = u // NQ
            qi = u % NQ
            hrow = pl.multiple_of(h * HP, HP)
            mt = m_of(t)
            p = jnp.exp2(s_ring[t % RING][...] - mt).astype(_BF16)
            pv = _dot(vt_v[pl.ds(hrow, HP), kc * TK:(kc + 1) * TK], p)
            if kc == 0:
                acc = pv
            else:
                acc = acc * jnp.exp2(m_of(t - 1) - mt) + pv
            if kc == NK - 1:
                qoff = pl.multiple_of(qi * TQ, TQ)
                o = acc / acc[DH:DH + 1, :]
                ot_v[pl.ds(hrow, HP), pl.ds(qoff, TQ)] = o.astype(_BF16)
        return carry

    jax.lax.fori_loop(0, NU // UNITS, attn_body, 0)

    for c in range(S // TS3):
        cols = slice(c * TS3, (c + 1) * TS3)
        ht = ht_v[:, cols] + _dot(wo_t[...], ot_v[:, cols])
        ht_v[:, cols] = ht
        mu = jnp.mean(ht, axis=0, keepdims=True)
        hc = ht - mu
        var = jnp.mean(hc * hc, axis=0, keepdims=True)
        hnt_v[:, cols] = (hc * jax.lax.rsqrt(var + EPS)).astype(_BF16)

    w1_copy.wait()
    b1_copy.wait()
    for c in range(F // TF4):
        cols = slice(c * TF4, (c + 1) * TF4)
        u = _dot(hnt_v[...], w1_v[:, cols]) + b1_v[:, cols].astype(_F32)
        g_v[:, cols] = jax.nn.gelu(u, approximate=True).astype(_BF16)

    w2_copy.wait()
    b2_copy.wait()
    for c in range(N5):
        cols = slice(c * TS5, (c + 1) * TS5)
        y = _dot(g_v[...], w2_v[:, cols]) + b2_v[:, cols].astype(_F32) + ht_v[:, cols]
        out_v[cols, :] = y.astype(_BF16).T
        out_copy(c).start()
    for c in range(N5):
        out_copy(c).wait()


@jax.jit
def pallas_sequential_preLN__mha_block__mixer_token_mlp__prompt_kernel(
    A_x: jax.Array,
    A_wqkv: jax.Array,
    A_wo: jax.Array,
    B_x: jax.Array,
    B_w1: jax.Array,
    B_b1: jax.Array,
    B_w2: jax.Array,
    B_b2: jax.Array,
):
    del B_x
    x = A_x.reshape(S, D)
    b1 = B_b1.reshape(1, F)
    b2 = B_b2.reshape(1, S)

    scratch = [
        pltpu.VMEM((S, D), _BF16),
        pltpu.VMEM((D, 3 * D), _BF16),
        pltpu.VMEM((D, D), _BF16),
        pltpu.VMEM((S, F), _BF16),
        pltpu.VMEM((1, F), _BF16),
        pltpu.VMEM((F, S), _BF16),
        pltpu.VMEM((1, S), _BF16),
        pltpu.VMEM((NG, D, GW), _BF16),
        pltpu.VMEM((D + H * HP, D), _BF16),
        pltpu.VMEM((D, H * HP), _BF16),
        pltpu.VMEM((NG, S, GW), _BF16),
        pltpu.VMEM((NG, GW, S), _BF16),
        pltpu.VMEM((H * HP, S), _BF16),
        pltpu.VMEM((H * HP, S), _BF16),
        pltpu.VMEM((D, S), _F32),
        pltpu.VMEM((D, S), _BF16),
        pltpu.VMEM((D, F), _BF16),
        pltpu.VMEM((S, D), _BF16),
        pltpu.SemaphoreType.DMA((NSEM,)),
    ]
    scratch += [pltpu.VMEM((TK, TQ), _F32)] * RING
    scratch += [pltpu.VMEM((1, TQ), _F32)] * RING

    any_spec = pl.BlockSpec(memory_space=pl.ANY)
    out = pl.pallas_call(
        _kernel,
        out_shape=jax.ShapeDtypeStruct((S, D), _BF16),
        in_specs=[any_spec] * 7,
        out_specs=any_spec,
        scratch_shapes=scratch,
        compiler_params=pltpu.CompilerParams(vmem_limit_bytes=100 * 1024 * 1024),
    )(x, A_wqkv, A_wo, B_w1, b1, B_w2, b2)
    return out.reshape(1, S, D)
```

```python
import functools
import math

import jax
import jax.numpy as jnp
import jax.experimental.pallas as pl
import jax.experimental.pallas.tpu as pltpu

S = 2048
D = 448
H = 16
DH = 28
F = 1792
HPG = 4
NG = H // HPG
GW = HPG * DH
HP = 32
EPS = 1e-5

TS1 = 512
TQ = 512
TK = 128
LOOKAHEAD = 2
UNITS = 8
TS3 = 512
TF4 = 256
TS5 = 256

NQ = S // TQ
NK = S // TK
NU = H * NQ
STEPS = UNITS * NK
RING = LOOKAHEAD + 1
while STEPS % RING:
    RING += 1

N1 = S // TS1
N5 = S // TS5

SEM_X = 0
SEM_WQKV = SEM_X + N1
SEM_WO = SEM_WQKV + 1
SEM_B1 = SEM_WO + 1
SEM_B2 = SEM_B1 + 1
SEM_W1 = SEM_B2 + 1
SEM_W2 = SEM_W1 + 1
SEM_OUT = SEM_W2 + 1
NSEM = SEM_OUT + N5

_NT = (((1,), (1,)), ((), ()))
_F32 = jnp.float32
_BF16 = jnp.bfloat16


def _dot(a, b):
    return jnp.dot(a, b, preferred_element_type=_F32)


def _dot_nt(a, b):
    return jax.lax.dot_general(a, b, _NT, preferred_element_type=_F32)


def _pad_head_rows(w):
    zeros = jnp.zeros((HP - DH, w.shape[1]), w.dtype)
    parts = []
    for h in range(H):
        parts.append(w[h * DH:(h + 1) * DH, :])
        parts.append(zeros)
    return jnp.concatenate(parts, axis=0)


def _kernel(xt_hbm, wqkv_hbm, wo_hbm, w1_hbm, b1_hbm, w2_hbm, b2_hbm, out_hbm,
            xt_v, wqkv_v, wo_v, w1_v, b1_v, w2_v, b2_v,
            w_t, wo_t, k_v, qt_v, vt_v, ot_v, ht_v, hnt_v, g_v, out_v,
            sems, *ring):
    s_ring = ring[:RING]
    m_ring = ring[RING:]

    def copy(src, dst, sem):
        return pltpu.make_async_copy(src, dst, sems.at[sem])

    def x_copy(c):
        cols = pl.ds(c * TS1, TS1)
        return copy(xt_hbm.at[:, cols], xt_v.at[:, cols], SEM_X + c)

    def out_copy(c):
        cols = pl.ds(c * TS5, TS5)
        return copy(out_v.at[:, cols], out_hbm.at[:, cols], SEM_OUT + c)

    wqkv_copy = copy(wqkv_hbm, wqkv_v, SEM_WQKV)
    wo_copy = copy(wo_hbm, wo_v, SEM_WO)
    b1_copy = copy(b1_hbm, b1_v, SEM_B1)
    b2_copy = copy(b2_hbm, b2_v, SEM_B2)
    w1_copy = copy(w1_hbm, w1_v, SEM_W1)
    w2_copy = copy(w2_hbm, w2_v, SEM_W2)

    wqkv_copy.start()
    for c in range(N1):
        x_copy(c).start()
    wo_copy.start()
    b1_copy.start()
    b2_copy.start()

    wqkv_copy.wait()
    w_t[0:2 * D, :] = wqkv_v[:, 0:2 * D].T
    wv_t = wqkv_v[:, 2 * D:3 * D].astype(_F32).T
    w_t[2 * D:, :] = _pad_head_rows(wv_t).astype(_BF16)

    q_scale = (DH ** -0.5) * math.log2(math.e)
    for c in range(N1):
        x_copy(c).wait()
        if c == N1 - 1:
            w1_copy.start()
            w2_copy.start()
        cols = slice(c * TS1, (c + 1) * TS1)
        xf = xt_v[:, cols].astype(_F32)
        mu = jnp.mean(xf, axis=0, keepdims=True)
        xc = xf - mu
        var = jnp.mean(xc * xc, axis=0, keepdims=True)
        xn = (xc * jax.lax.rsqrt(var + EPS)).astype(_BF16)
        qkv = _dot(w_t[...], xn)
        for g in range(NG):
            qt_v[g, :, cols] = (qkv[g * GW:(g + 1) * GW, :] * q_scale).astype(_BF16)
            k_v[g, cols, :] = qkv[D + g * GW:D + (g + 1) * GW, :].astype(_BF16).T
        vt = qkv[2 * D:, :]
        rid = jax.lax.broadcasted_iota(jnp.int32, vt.shape, 0)
        vt = jnp.where(rid % HP == DH, 1.0, vt)
        vt_v[:, cols] = vt.astype(_BF16)

    wo_copy.wait()
    wo_t[...] = _pad_head_rows(wo_v[...].astype(_F32)).astype(_BF16).T

    def get_wq(u):
        h = u // NQ
        qi = u % NQ
        g = h // HPG
        j = h % HPG
        qoff = pl.multiple_of(qi * TQ, TQ)
        wq = qt_v[g, :, pl.ds(qoff, TQ)]
        rid = jax.lax.broadcasted_iota(jnp.int32, (GW, TQ), 0)
        keep = (rid >= DH * j) & (rid < DH * j + DH)
        return jnp.where(keep, wq, jnp.zeros_like(wq)), g

    def score_chunk(slot, g, wq, kc, m_prev):
        s = _dot(k_v[g, kc * TK:(kc + 1) * TK, :], wq)
        s_ring[slot][...] = s
        cm = jnp.max(jnp.max(s.reshape(TK // 8, 8, TQ), axis=0), axis=0, keepdims=True)
        m = cm if m_prev is None else jnp.maximum(m_prev, cm)
        m_ring[slot][...] = m
        return m

    wq0, g0 = get_wq(0)
    m0 = None
    for t in range(LOOKAHEAD):
        m0 = score_chunk(t % RING, g0, wq0, t, m0)

    def attn_body(i, carry):
        u0 = i * UNITS
        wqs = {}
        ms = {}

        def wq_of(ul):
            if ul not in wqs:
                wqs[ul] = get_wq(jnp.minimum(u0 + ul, NU - 1))
            return wqs[ul]

        def m_of(t):
            if t not in ms:
                ms[t] = m_ring[t % RING][...]
            return ms[t]

        acc = None
        for t in range(STEPS):
            ta = t + LOOKAHEAD
            ul, kc = divmod(ta, NK)
            wq, g = wq_of(ul)
            ms[ta] = score_chunk(ta % RING, g, wq, kc, None if kc == 0 else m_of(ta - 1))
            ul, kc = divmod(t, NK)
            u = u0 + ul
            h = u // NQ
            qi = u % NQ
            hrow = pl.multiple_of(h * HP, HP)
            mt = m_of(t)
            p = jnp.exp2(s_ring[t % RING][...] - mt).astype(_BF16)
            pv = _dot(vt_v[pl.ds(hrow, HP), kc * TK:(kc + 1) * TK], p)
            if kc == 0:
                acc = pv
            else:
                acc = acc * jnp.exp2(m_of(t - 1) - mt) + pv
            if kc == NK - 1:
                qoff = pl.multiple_of(qi * TQ, TQ)
                o = acc / acc[DH:DH + 1, :]
                ot_v[pl.ds(hrow, HP), pl.ds(qoff, TQ)] = o.astype(_BF16)
        return carry

    jax.lax.fori_loop(0, NU // UNITS, attn_body, 0)

    for c in range(S // TS3):
        cols = slice(c * TS3, (c + 1) * TS3)
        ht = xt_v[:, cols].astype(_F32) + _dot(wo_t[...], ot_v[:, cols])
        ht_v[:, cols] = ht
        mu = jnp.mean(ht, axis=0, keepdims=True)
        hc = ht - mu
        var = jnp.mean(hc * hc, axis=0, keepdims=True)
        hnt_v[:, cols] = (hc * jax.lax.rsqrt(var + EPS)).astype(_BF16)

    w1_copy.wait()
    b1_copy.wait()
    for c in range(F // TF4):
        cols = slice(c * TF4, (c + 1) * TF4)
        u = _dot(hnt_v[...], w1_v[:, cols]) + b1_v[:, cols].astype(_F32)
        g_v[:, cols] = jax.nn.gelu(u, approximate=True).astype(_BF16)

    w2_copy.wait()
    b2_copy.wait()
    for c in range(N5):
        cols = slice(c * TS5, (c + 1) * TS5)
        y = _dot(g_v[...], w2_v[:, cols]) + b2_v[:, cols].astype(_F32) + ht_v[:, cols]
        out_v[:, cols] = y.astype(_BF16)
        out_copy(c).start()
    for c in range(N5):
        out_copy(c).wait()


@jax.jit
def pallas_sequential_preLN__mha_block__mixer_token_mlp__prompt_kernel(
    A_x: jax.Array,
    A_wqkv: jax.Array,
    A_wo: jax.Array,
    B_x: jax.Array,
    B_w1: jax.Array,
    B_b1: jax.Array,
    B_w2: jax.Array,
    B_b2: jax.Array,
):
    del B_x
    xt = jnp.transpose(A_x, (0, 2, 1)).reshape(D, S)
    b1 = B_b1.reshape(1, F)
    b2 = B_b2.reshape(1, S)

    scratch = [
        pltpu.VMEM((D, S), _BF16),
        pltpu.VMEM((D, 3 * D), _BF16),
        pltpu.VMEM((D, D), _BF16),
        pltpu.VMEM((S, F), _BF16),
        pltpu.VMEM((1, F), _BF16),
        pltpu.VMEM((F, S), _BF16),
        pltpu.VMEM((1, S), _BF16),
        pltpu.VMEM((2 * D + H * HP, D), _BF16),
        pltpu.VMEM((D, H * HP), _BF16),
        pltpu.VMEM((NG, S, GW), _BF16),
        pltpu.VMEM((NG, GW, S), _BF16),
        pltpu.VMEM((H * HP, S), _BF16),
        pltpu.VMEM((H * HP, S), _BF16),
        pltpu.VMEM((D, S), _F32),
        pltpu.VMEM((D, S), _BF16),
        pltpu.VMEM((D, F), _BF16),
        pltpu.VMEM((D, S), _BF16),
        pltpu.SemaphoreType.DMA((NSEM,)),
    ]
    scratch += [pltpu.VMEM((TK, TQ), _F32)] * RING
    scratch += [pltpu.VMEM((1, TQ), _F32)] * RING

    any_spec = pl.BlockSpec(memory_space=pl.ANY)
    out = pl.pallas_call(
        _kernel,
        out_shape=jax.ShapeDtypeStruct((D, S), _BF16),
        in_specs=[any_spec] * 7,
        out_specs=any_spec,
        scratch_shapes=scratch,
        compiler_params=pltpu.CompilerParams(vmem_limit_bytes=100 * 1024 * 1024),
    )(xt, A_wqkv, A_wo, B_w1, b1, B_w2, b2)
    return jnp.transpose(out.reshape(1, D, S), (0, 2, 1))
```

```python
import functools
import math

import jax
import jax.numpy as jnp
import jax.experimental.pallas as pl
import jax.experimental.pallas.tpu as pltpu

S = 2048
D = 448
H = 16
DH = 28
F = 1792
HPG = 4
NG = H // HPG
GW = HPG * DH
GP = 128
HP = 32
EPS = 1e-5

TS1 = 512
TQ = 512
TK = 128
LOOKAHEAD = 2
UNITS = 8
TS3 = 512
TF4 = 256
TS5 = 256

NQ = S // TQ
NK = S // TK
NU = H * NQ
STEPS = UNITS * NK
RING = LOOKAHEAD + 1
while STEPS % RING:
    RING += 1

N1 = S // TS1
X_PIECES = ((0, 1), (1, 2), (2, N1))
N5 = S // TS5

SEM_X = 0
SEM_WQKV = SEM_X + len(X_PIECES)
SEM_WO = SEM_WQKV + 1
SEM_B1 = SEM_WO + 1
SEM_B2 = SEM_B1 + 1
SEM_W1 = SEM_B2 + 1
SEM_W2 = SEM_W1 + 1
SEM_OUT = SEM_W2 + 1
NSEM = SEM_OUT + N5

_NT = (((1,), (1,)), ((), ()))
_F32 = jnp.float32
_BF16 = jnp.bfloat16


def _dot(a, b):
    return jnp.dot(a, b, preferred_element_type=_F32)


def _dot_nt(a, b):
    return jax.lax.dot_general(a, b, _NT, preferred_element_type=_F32)


def _pad_head_rows(w):
    zeros = jnp.zeros((HP - DH, w.shape[1]), w.dtype)
    parts = []
    for h in range(H):
        parts.append(w[h * DH:(h + 1) * DH, :])
        parts.append(zeros)
    return jnp.concatenate(parts, axis=0)


def _kernel(xt_hbm, wqkv_hbm, wo_hbm, w1_hbm, b1_hbm, w2_hbm, b2_hbm, out_hbm,
            xt_v, wqkv_v, wo_v, w1_v, b1_v, w2_v, b2_v,
            w_t, wo_t, k_v, qt_v, vt_v, ot_v, ht_v, hnt_v, g_v, out_v,
            sems, *ring):
    s_ring = ring[:RING]
    m_ring = ring[RING:]

    def copy(src, dst, sem):
        return pltpu.make_async_copy(src, dst, sems.at[sem])

    def x_copy(i):
        lo, hi = X_PIECES[i]
        cols = pl.ds(lo * TS1, (hi - lo) * TS1)
        return copy(xt_hbm.at[:, cols], xt_v.at[:, cols], SEM_X + i)

    def out_copy(c):
        cols = pl.ds(c * TS5, TS5)
        return copy(out_v.at[:, cols], out_hbm.at[:, cols], SEM_OUT + c)

    wqkv_copy = copy(wqkv_hbm, wqkv_v, SEM_WQKV)
    wo_copy = copy(wo_hbm, wo_v, SEM_WO)
    b1_copy = copy(b1_hbm, b1_v, SEM_B1)
    b2_copy = copy(b2_hbm, b2_v, SEM_B2)
    w1_copy = copy(w1_hbm, w1_v, SEM_W1)
    w2_copy = copy(w2_hbm, w2_v, SEM_W2)

    wqkv_copy.start()
    for i in range(len(X_PIECES)):
        x_copy(i).start()
    wo_copy.start()
    b1_copy.start()
    b2_copy.start()

    q_scale = (DH ** -0.5) * math.log2(math.e)

    def ln1(c):
        cols = slice(c * TS1, (c + 1) * TS1)
        xf = xt_v[:, cols].astype(_F32)
        mu = jnp.mean(xf, axis=0, keepdims=True)
        xc = xf - mu
        var = jnp.mean(xc * xc, axis=0, keepdims=True)
        return (xc * jax.lax.rsqrt(var + EPS)).astype(_BF16)

    def project(c, xn):
        cols = slice(c * TS1, (c + 1) * TS1)
        qkv = _dot(w_t[...], xn)
        zpad = jnp.zeros((GP - GW, TS1), _BF16)
        for g in range(NG):
            qg = (qkv[g * GW:(g + 1) * GW, :] * q_scale).astype(_BF16)
            qt_v[g, :, cols] = jnp.concatenate([qg, zpad], axis=0)
            kg = qkv[D + g * GW:D + (g + 1) * GW, :].astype(_BF16)
            k_v[g, cols, :] = jnp.concatenate([kg, zpad], axis=0).T
        vt = qkv[2 * D:, :]
        rid = jax.lax.broadcasted_iota(jnp.int32, vt.shape, 0)
        vt = jnp.where(rid % HP == DH, 1.0, vt)
        vt_v[:, cols] = vt.astype(_BF16)

    wqkv_copy.wait()
    x_copy(0).wait()
    w_t[0:2 * D, :] = wqkv_v[:, 0:2 * D].T
    wv_t = wqkv_v[:, 2 * D:3 * D].astype(_F32).T
    w_t[2 * D:, :] = _pad_head_rows(wv_t).astype(_BF16)
    xns = {}
    for i, (lo, hi) in enumerate(X_PIECES):
        if i > 0:
            x_copy(i).wait()
        if i == len(X_PIECES) - 1:
            w1_copy.start()
            w2_copy.start()
        for c in range(lo, hi):
            xns[c] = ln1(c)
            if c > 0:
                project(c - 1, xns.pop(c - 1))
    project(N1 - 1, xns.pop(N1 - 1))

    wo_copy.wait()
    wo_t[...] = _pad_head_rows(wo_v[...].astype(_F32)).astype(_BF16).T

    def get_wq(u):
        h = u // NQ
        qi = u % NQ
        g = h // HPG
        j = h % HPG
        qoff = pl.multiple_of(qi * TQ, TQ)
        wq = qt_v[g, :, pl.ds(qoff, TQ)]
        rid = jax.lax.broadcasted_iota(jnp.int32, (GP, TQ), 0)
        keep = (rid >= DH * j) & (rid < DH * j + DH)
        return jnp.where(keep, wq, jnp.zeros_like(wq)), g

    def score_chunk(slot, g, wq, kc, m_prev):
        s = _dot(k_v[g, kc * TK:(kc + 1) * TK, :], wq)
        s_ring[slot][...] = s
        cm = jnp.max(jnp.max(s.reshape(TK // 8, 8, TQ), axis=0), axis=0, keepdims=True)
        m = cm if m_prev is None else jnp.maximum(m_prev, cm)
        m_ring[slot][...] = m
        return m

    wq0, g0 = get_wq(0)
    m0 = None
    for t in range(LOOKAHEAD):
        m0 = score_chunk(t % RING, g0, wq0, t, m0)

    def attn_body(i, carry):
        u0 = i * UNITS
        wqs = {}
        ms = {}

        def wq_of(ul):
            if ul not in wqs:
                wqs[ul] = get_wq(jnp.minimum(u0 + ul, NU - 1))
            return wqs[ul]

        def m_of(t):
            if t not in ms:
                ms[t] = m_ring[t % RING][...]
            return ms[t]

        acc = None
        for t in range(STEPS):
            ta = t + LOOKAHEAD
            ul, kc = divmod(ta, NK)
            wq, g = wq_of(ul)
            ms[ta] = score_chunk(ta % RING, g, wq, kc, None if kc == 0 else m_of(ta - 1))
            ul, kc = divmod(t, NK)
            u = u0 + ul
            h = u // NQ
            qi = u % NQ
            hrow = pl.multiple_of(h * HP, HP)
            mt = m_of(t)
            p = jnp.exp2(s_ring[t % RING][...] - mt).astype(_BF16)
            pv = _dot(vt_v[pl.ds(hrow, HP), kc * TK:(kc + 1) * TK], p)
            if kc == 0:
                acc = pv
            else:
                acc = acc * jnp.exp2(m_of(t - 1) - mt) + pv
            if kc == NK - 1:
                qoff = pl.multiple_of(qi * TQ, TQ)
                o = acc / acc[DH:DH + 1, :]
                ot_v[pl.ds(hrow, HP), pl.ds(qoff, TQ)] = o.astype(_BF16)
        return carry

    jax.lax.fori_loop(0, NU // UNITS, attn_body, 0)

    for c in range(S // TS3):
        cols = slice(c * TS3, (c + 1) * TS3)
        ht = xt_v[:, cols].astype(_F32) + _dot(wo_t[...], ot_v[:, cols])
        ht_v[:, cols] = ht
        mu = jnp.mean(ht, axis=0, keepdims=True)
        hc = ht - mu
        var = jnp.mean(hc * hc, axis=0, keepdims=True)
        hnt_v[:, cols] = (hc * jax.lax.rsqrt(var + EPS)).astype(_BF16)

    w1_copy.wait()
    b1_copy.wait()
    for c in range(F // TF4):
        cols = slice(c * TF4, (c + 1) * TF4)
        u = _dot(hnt_v[...], w1_v[:, cols]) + b1_v[:, cols].astype(_F32)
        g_v[:, cols] = jax.nn.gelu(u, approximate=True).astype(_BF16)

    w2_copy.wait()
    b2_copy.wait()
    for c in range(N5):
        cols = slice(c * TS5, (c + 1) * TS5)
        y = _dot(g_v[...], w2_v[:, cols]) + b2_v[:, cols].astype(_F32) + ht_v[:, cols]
        out_v[:, cols] = y.astype(_BF16)
        out_copy(c).start()
    for c in range(N5):
        out_copy(c).wait()


@jax.jit
def pallas_sequential_preLN__mha_block__mixer_token_mlp__prompt_kernel(
    A_x: jax.Array,
    A_wqkv: jax.Array,
    A_wo: jax.Array,
    B_x: jax.Array,
    B_w1: jax.Array,
    B_b1: jax.Array,
    B_w2: jax.Array,
    B_b2: jax.Array,
):
    del B_x
    xt = jnp.transpose(A_x, (0, 2, 1)).reshape(D, S)
    b1 = B_b1.reshape(1, F)
    b2 = B_b2.reshape(1, S)

    scratch = [
        pltpu.VMEM((D, S), _BF16),
        pltpu.VMEM((D, 3 * D), _BF16),
        pltpu.VMEM((D, D), _BF16),
        pltpu.VMEM((S, F), _BF16),
        pltpu.VMEM((1, F), _BF16),
        pltpu.VMEM((F, S), _BF16),
        pltpu.VMEM((1, S), _BF16),
        pltpu.VMEM((2 * D + H * HP, D), _BF16),
        pltpu.VMEM((D, H * HP), _BF16),
        pltpu.VMEM((NG, S, GP), _BF16),
        pltpu.VMEM((NG, GP, S), _BF16),
        pltpu.VMEM((H * HP, S), _BF16),
        pltpu.VMEM((H * HP, S), _BF16),
        pltpu.VMEM((D, S), _F32),
        pltpu.VMEM((D, S), _BF16),
        pltpu.VMEM((D, F), _BF16),
        pltpu.VMEM((D, S), _BF16),
        pltpu.SemaphoreType.DMA((NSEM,)),
    ]
    scratch += [pltpu.VMEM((TK, TQ), _F32)] * RING
    scratch += [pltpu.VMEM((1, TQ), _F32)] * RING

    any_spec = pl.BlockSpec(memory_space=pl.ANY)
    out = pl.pallas_call(
        _kernel,
        out_shape=jax.ShapeDtypeStruct((D, S), _BF16),
        in_specs=[any_spec] * 7,
        out_specs=any_spec,
        scratch_shapes=scratch,
        compiler_params=pltpu.CompilerParams(vmem_limit_bytes=100 * 1024 * 1024),
    )(xt, A_wqkv, A_wo, B_w1, b1, B_w2, b2)
    return jnp.transpose(out.reshape(1, D, S), (0, 2, 1))
```

```python
import functools
import math

import jax
import jax.numpy as jnp
import jax.experimental.pallas as pl
import jax.experimental.pallas.tpu as pltpu

S = 2048
D = 448
H = 16
DH = 28
F = 1792
HPG = 4
NG = H // HPG
GW = HPG * DH
GP = 128
HP = 32
EPS = 1e-5

X_OFFS = (0, 512, 1024, 1536, 2048)
TQ = 512
TK = 128
LOOKAHEAD = 2
UNITS = 8
TS3 = 512
TF4 = 256
TS5 = 256

NQ = S // TQ
NK = S // TK
NU = H * NQ
STEPS = UNITS * NK
RING = LOOKAHEAD + 1
while STEPS % RING:
    RING += 1

N1 = len(X_OFFS) - 1
X_PIECES = ((0, X_OFFS[1]), (X_OFFS[1], S))
N5 = S // TS5

SEM_X = 0
SEM_WQKV = SEM_X + len(X_PIECES)
SEM_WO = SEM_WQKV + 1
SEM_B1 = SEM_WO + 1
SEM_B2 = SEM_B1 + 1
SEM_W1 = SEM_B2 + 1
SEM_W2 = SEM_W1 + 1
SEM_OUT = SEM_W2 + 1
NSEM = SEM_OUT + N5

_NT = (((1,), (1,)), ((), ()))
_F32 = jnp.float32
_BF16 = jnp.bfloat16


def _dot(a, b):
    return jnp.dot(a, b, preferred_element_type=_F32)


def _dot_nt(a, b):
    return jax.lax.dot_general(a, b, _NT, preferred_element_type=_F32)


def _pad_head_rows(w):
    zeros = jnp.zeros((HP - DH, w.shape[1]), w.dtype)
    parts = []
    for h in range(H):
        parts.append(w[h * DH:(h + 1) * DH, :])
        parts.append(zeros)
    return jnp.concatenate(parts, axis=0)


def _kernel(xt_hbm, wqkv_hbm, wo_hbm, w1_hbm, b1_hbm, w2_hbm, b2_hbm, out_hbm,
            xt_v, wqkv_v, wo_v, w1_v, b1_v, w2_v, b2_v,
            w_t, wo_t, k_v, qt_v, vt_v, ot_v, ht_v, hnt_v, g_v, out_v,
            sems, *ring):
    s_ring = ring[:RING]
    m_ring = ring[RING:]

    def copy(src, dst, sem):
        return pltpu.make_async_copy(src, dst, sems.at[sem])

    def x_copy(i):
        lo, hi = X_PIECES[i]
        cols = pl.ds(lo, hi - lo)
        return copy(xt_hbm.at[:, cols], xt_v.at[:, cols], SEM_X + i)

    def out_copy(c):
        cols = pl.ds(c * TS5, TS5)
        return copy(out_v.at[:, cols], out_hbm.at[:, cols], SEM_OUT + c)

    wqkv_copy = copy(wqkv_hbm, wqkv_v, SEM_WQKV)
    wo_copy = copy(wo_hbm, wo_v, SEM_WO)
    b1_copy = copy(b1_hbm, b1_v, SEM_B1)
    b2_copy = copy(b2_hbm, b2_v, SEM_B2)
    w1_copy = copy(w1_hbm, w1_v, SEM_W1)
    w2_copy = copy(w2_hbm, w2_v, SEM_W2)

    wqkv_copy.start()
    x_copy(0).start()

    q_scale = (DH ** -0.5) * math.log2(math.e)

    def ln1(c):
        cols = slice(X_OFFS[c], X_OFFS[c + 1])
        xf = xt_v[:, cols].astype(_F32)
        mu = jnp.mean(xf, axis=0, keepdims=True)
        xc = xf - mu
        var = jnp.mean(xc * xc, axis=0, keepdims=True)
        return (xc * jax.lax.rsqrt(var + EPS)).astype(_BF16)

    def project_qk(c, xn):
        cols = slice(X_OFFS[c], X_OFFS[c + 1])
        qk = _dot(w_t[0:2 * D, :], xn)
        zpad = jnp.zeros((GP - GW, xn.shape[1]), _BF16)
        for g in range(NG):
            qg = (qk[g * GW:(g + 1) * GW, :] * q_scale).astype(_BF16)
            qt_v[g, :, cols] = jnp.concatenate([qg, zpad], axis=0)
            kg = qk[D + g * GW:D + (g + 1) * GW, :].astype(_BF16)
            k_v[g, cols, :] = jnp.concatenate([kg, zpad], axis=0).T

    def project_v(c, xn):
        cols = slice(X_OFFS[c], X_OFFS[c + 1])
        vt = _dot(w_t[2 * D:, :], xn)
        rid = jax.lax.broadcasted_iota(jnp.int32, vt.shape, 0)
        vt = jnp.where(rid % HP == DH, 1.0, vt)
        vt_v[:, cols] = vt.astype(_BF16)

    wqkv_copy.wait()
    x_copy(0).wait()
    x_copy(1).start()
    wo_copy.start()
    b1_copy.start()
    b2_copy.start()
    w_t[0:2 * D, :] = wqkv_v[:, 0:2 * D].T
    wv_t = wqkv_v[:, 2 * D:3 * D].astype(_F32).T
    w_t[2 * D:, :] = _pad_head_rows(wv_t).astype(_BF16)
    xn = ln1(0)
    project_qk(0, xn)
    x_copy(1).wait()
    w1_copy.start()
    w2_copy.start()
    for c in range(1, N1):
        xn_next = ln1(c)
        project_v(c - 1, xn)
        project_qk(c, xn_next)
        xn = xn_next
    project_v(N1 - 1, xn)

    wo_copy.wait()
    wo_t[...] = _pad_head_rows(wo_v[...].astype(_F32)).astype(_BF16).T

    def get_wq(u):
        h = u // NQ
        qi = u % NQ
        g = h // HPG
        j = h % HPG
        qoff = pl.multiple_of(qi * TQ, TQ)
        wq = qt_v[g, :, pl.ds(qoff, TQ)]
        rid = jax.lax.broadcasted_iota(jnp.int32, (GP, TQ), 0)
        keep = (rid >= DH * j) & (rid < DH * j + DH)
        return jnp.where(keep, wq, jnp.zeros_like(wq)), g

    def score_chunk(slot, g, wq, kc, m_prev):
        s = _dot(k_v[g, kc * TK:(kc + 1) * TK, :], wq)
        s_ring[slot][...] = s
        cm = jnp.max(jnp.max(s.reshape(TK // 8, 8, TQ), axis=0), axis=0, keepdims=True)
        m = cm if m_prev is None else jnp.maximum(m_prev, cm)
        m_ring[slot][...] = m
        return m

    wq0, g0 = get_wq(0)
    m0 = None
    for t in range(LOOKAHEAD):
        m0 = score_chunk(t % RING, g0, wq0, t, m0)

    def attn_body(i, carry):
        u0 = i * UNITS
        wqs = {}
        ms = {}

        def wq_of(ul):
            if ul not in wqs:
                wqs[ul] = get_wq(jnp.minimum(u0 + ul, NU - 1))
            return wqs[ul]

        def m_of(t):
            if t not in ms:
                ms[t] = m_ring[t % RING][...]
            return ms[t]

        acc = None
        for t in range(STEPS):
            ta = t + LOOKAHEAD
            ul, kc = divmod(ta, NK)
            wq, g = wq_of(ul)
            ms[ta] = score_chunk(ta % RING, g, wq, kc, None if kc == 0 else m_of(ta - 1))
            ul, kc = divmod(t, NK)
            u = u0 + ul
            h = u // NQ
            qi = u % NQ
            hrow = pl.multiple_of(h * HP, HP)
            mt = m_of(t)
            p = jnp.exp2(s_ring[t % RING][...] - mt).astype(_BF16)
            pv = _dot(vt_v[pl.ds(hrow, HP), kc * TK:(kc + 1) * TK], p)
            if kc == 0:
                acc = pv
            else:
                acc = acc * jnp.exp2(m_of(t - 1) - mt) + pv
            if kc == NK - 1:
                qoff = pl.multiple_of(qi * TQ, TQ)
                o = acc / acc[DH:DH + 1, :]
                ot_v[pl.ds(hrow, HP), pl.ds(qoff, TQ)] = o.astype(_BF16)
        return carry

    jax.lax.fori_loop(0, NU // UNITS, attn_body, 0)

    for c in range(S // TS3):
        cols = slice(c * TS3, (c + 1) * TS3)
        ht = xt_v[:, cols].astype(_F32) + _dot(wo_t[...], ot_v[:, cols])
        ht_v[:, cols] = ht
        mu = jnp.mean(ht, axis=0, keepdims=True)
        hc = ht - mu
        var = jnp.mean(hc * hc, axis=0, keepdims=True)
        hnt_v[:, cols] = (hc * jax.lax.rsqrt(var + EPS)).astype(_BF16)

    w1_copy.wait()
    b1_copy.wait()
    for c in range(F // TF4):
        cols = slice(c * TF4, (c + 1) * TF4)
        u = _dot(hnt_v[...], w1_v[:, cols]) + b1_v[:, cols].astype(_F32)
        g_v[:, cols] = jax.nn.gelu(u, approximate=True).astype(_BF16)

    w2_copy.wait()
    b2_copy.wait()
    for c in range(N5):
        cols = slice(c * TS5, (c + 1) * TS5)
        y = _dot(g_v[...], w2_v[:, cols]) + b2_v[:, cols].astype(_F32) + ht_v[:, cols]
        out_v[:, cols] = y.astype(_BF16)
        out_copy(c).start()
    for c in range(N5):
        out_copy(c).wait()


@jax.jit
def pallas_sequential_preLN__mha_block__mixer_token_mlp__prompt_kernel(
    A_x: jax.Array,
    A_wqkv: jax.Array,
    A_wo: jax.Array,
    B_x: jax.Array,
    B_w1: jax.Array,
    B_b1: jax.Array,
    B_w2: jax.Array,
    B_b2: jax.Array,
):
    del B_x
    xt = jnp.transpose(A_x, (0, 2, 1)).reshape(D, S)
    b1 = B_b1.reshape(1, F)
    b2 = B_b2.reshape(1, S)

    scratch = [
        pltpu.VMEM((D, S), _BF16),
        pltpu.VMEM((D, 3 * D), _BF16),
        pltpu.VMEM((D, D), _BF16),
        pltpu.VMEM((S, F), _BF16),
        pltpu.VMEM((1, F), _BF16),
        pltpu.VMEM((F, S), _BF16),
        pltpu.VMEM((1, S), _BF16),
        pltpu.VMEM((2 * D + H * HP, D), _BF16),
        pltpu.VMEM((D, H * HP), _BF16),
        pltpu.VMEM((NG, S, GP), _BF16),
        pltpu.VMEM((NG, GP, S), _BF16),
        pltpu.VMEM((H * HP, S), _BF16),
        pltpu.VMEM((H * HP, S), _BF16),
        pltpu.VMEM((D, S), _F32),
        pltpu.VMEM((D, S), _BF16),
        pltpu.VMEM((D, F), _BF16),
        pltpu.VMEM((D, S), _BF16),
        pltpu.SemaphoreType.DMA((NSEM,)),
    ]
    scratch += [pltpu.VMEM((TK, TQ), _F32)] * RING
    scratch += [pltpu.VMEM((1, TQ), _F32)] * RING

    any_spec = pl.BlockSpec(memory_space=pl.ANY)
    out = pl.pallas_call(
        _kernel,
        out_shape=jax.ShapeDtypeStruct((D, S), _BF16),
        in_specs=[any_spec] * 7,
        out_specs=any_spec,
        scratch_shapes=scratch,
        compiler_params=pltpu.CompilerParams(vmem_limit_bytes=100 * 1024 * 1024),
    )(xt, A_wqkv, A_wo, B_w1, b1, B_w2, b2)
    return jnp.transpose(out.reshape(1, D, S), (0, 2, 1))
```

```python
import functools
import math

import jax
import jax.numpy as jnp
import jax.experimental.pallas as pl
import jax.experimental.pallas.tpu as pltpu

S = 2048
D = 448
H = 16
DH = 28
F = 1792
HPG = 4
NG = H // HPG
GW = HPG * DH
GP = 128
HP = 32
EPS = 1e-5

X_OFFS = (0, 256, 768, 1280, 1792, 2048)
TQ = 1024
TK = 128
LOOKAHEAD = 2
UNITS = 8
TS3 = 512
TF4 = 256
TS5 = 256

NQ = S // TQ
NK = S // TK
NU = H * NQ
STEPS = UNITS * NK
RING = LOOKAHEAD + 1
while STEPS % RING:
    RING += 1

N1 = len(X_OFFS) - 1
X_PIECES = ((0, X_OFFS[1]), (X_OFFS[1], X_OFFS[2]), (X_OFFS[2], S))
W_PIECES = ((0, 512), (512, 2 * D), (2 * D, 3 * D))
N5 = S // TS5

SEM_X = 0
SEM_WQKV = SEM_X + len(X_PIECES)
SEM_WO = SEM_WQKV + len(W_PIECES)
SEM_B1 = SEM_WO + 1
SEM_B2 = SEM_B1 + 1
SEM_W1 = SEM_B2 + 1
SEM_W2 = SEM_W1 + 1
SEM_OUT = SEM_W2 + 1
NSEM = SEM_OUT + N5

_NT = (((1,), (1,)), ((), ()))
_F32 = jnp.float32
_BF16 = jnp.bfloat16


def _dot(a, b):
    return jnp.dot(a, b, preferred_element_type=_F32)


def _dot_nt(a, b):
    return jax.lax.dot_general(a, b, _NT, preferred_element_type=_F32)


def _pad_head_rows(w):
    zeros = jnp.zeros((HP - DH, w.shape[1]), w.dtype)
    parts = []
    for h in range(H):
        parts.append(w[h * DH:(h + 1) * DH, :])
        parts.append(zeros)
    return jnp.concatenate(parts, axis=0)


def _kernel(xt_hbm, wqkv_hbm, wo_hbm, w1_hbm, b1_hbm, w2_hbm, b2_hbm, out_hbm,
            xt_v, wqkv_v, wo_v, w1_v, b1_v, w2_v, b2_v,
            w_t, wo_t, k_v, qt_v, vt_v, ot_v, ht_v, hnt_v, g_v, out_v,
            sems, *ring):
    s_ring = ring[:RING]
    m_ring = ring[RING:]

    def copy(src, dst, sem):
        return pltpu.make_async_copy(src, dst, sems.at[sem])

    def x_copy(i):
        lo, hi = X_PIECES[i]
        cols = pl.ds(lo, hi - lo)
        return copy(xt_hbm.at[:, cols], xt_v.at[:, cols], SEM_X + i)

    def out_copy(c):
        cols = pl.ds(c * TS5, TS5)
        return copy(out_v.at[:, cols], out_hbm.at[:, cols], SEM_OUT + c)

    def w_copy(i):
        lo, hi = W_PIECES[i]
        cols = pl.ds(lo, hi - lo)
        return copy(wqkv_hbm.at[:, cols], wqkv_v.at[:, cols], SEM_WQKV + i)

    wo_copy = copy(wo_hbm, wo_v, SEM_WO)
    b1_copy = copy(b1_hbm, b1_v, SEM_B1)
    b2_copy = copy(b2_hbm, b2_v, SEM_B2)
    w1_copy = copy(w1_hbm, w1_v, SEM_W1)
    w2_copy = copy(w2_hbm, w2_v, SEM_W2)

    x_copy(0).start()
    w_copy(0).start()
    w_copy(1).start()
    w_copy(2).start()
    x_copy(1).start()
    x_copy(2).start()
    wo_copy.start()
    b1_copy.start()
    b2_copy.start()
    w1_copy.start()
    w2_copy.start()
    x_copy(0).wait()
    w_copy(0).wait()

    q_scale = (DH ** -0.5) * math.log2(math.e)

    def ln1(c):
        cols = slice(X_OFFS[c], X_OFFS[c + 1])
        xf = xt_v[:, cols].astype(_F32)
        mu = jnp.mean(xf, axis=0, keepdims=True)
        xc = xf - mu
        var = jnp.mean(xc * xc, axis=0, keepdims=True)
        return (xc * jax.lax.rsqrt(var + EPS)).astype(_BF16)

    def store_q(c, q):
        cols = slice(X_OFFS[c], X_OFFS[c + 1])
        zpad = jnp.zeros((GP - GW, q.shape[1]), _BF16)
        for g in range(NG):
            qg = (q[g * GW:(g + 1) * GW, :] * q_scale).astype(_BF16)
            qt_v[g, :, cols] = jnp.concatenate([qg, zpad], axis=0)

    def store_k(c, k):
        cols = slice(X_OFFS[c], X_OFFS[c + 1])
        zpad = jnp.zeros((GP - GW, k.shape[1]), _BF16)
        for g in range(NG):
            kg = k[g * GW:(g + 1) * GW, :].astype(_BF16)
            k_v[g, cols, :] = jnp.concatenate([kg, zpad], axis=0).T

    def project_qk(c, xn):
        qk = _dot(w_t[0:2 * D, :], xn)
        store_q(c, qk[0:D, :])
        store_k(c, qk[D:2 * D, :])

    def project_v(c, xn):
        cols = slice(X_OFFS[c], X_OFFS[c + 1])
        vt = _dot(w_t[2 * D:, :], xn)
        rid = jax.lax.broadcasted_iota(jnp.int32, vt.shape, 0)
        vt = jnp.where(rid % HP == DH, 1.0, vt)
        vt_v[:, cols] = vt.astype(_BF16)

    (a0, a1), (b0, b1), (c0, c1) = W_PIECES
    w_t[a0:a1, :] = wqkv_v[:, a0:a1].T
    xn = ln1(0)
    w_copy(1).wait()
    w_t[b0:b1, :] = wqkv_v[:, b0:b1].T
    ra = _dot(w_t[a0:a1, :], xn)
    store_q(0, ra[0:D, :])
    w_copy(2).wait()
    wv_t = wqkv_v[:, c0:c1].astype(_F32).T
    w_t[2 * D:, :] = _pad_head_rows(wv_t).astype(_BF16)
    rb = _dot(w_t[b0:b1, :], xn)
    store_k(0, jnp.concatenate([ra[D:, :], rb], axis=0))
    x_copy(1).wait()
    for c in range(1, N1):
        if c == 2:
            x_copy(2).wait()
            wo_copy.wait()
            wo_t[...] = _pad_head_rows(wo_v[...].astype(_F32)).astype(_BF16).T
        xn_next = ln1(c)
        project_v(c - 1, xn)
        project_qk(c, xn_next)
        xn = xn_next
    project_v(N1 - 1, xn)

    def get_wq(u):
        h = u // NQ
        qi = u % NQ
        g = h // HPG
        j = h % HPG
        qoff = pl.multiple_of(qi * TQ, TQ)
        wq = qt_v[g, :, pl.ds(qoff, TQ)]
        rid = jax.lax.broadcasted_iota(jnp.int32, (GP, TQ), 0)
        keep = (rid >= DH * j) & (rid < DH * j + DH)
        return jnp.where(keep, wq, jnp.zeros_like(wq)), g

    def score_chunk(slot, g, wq, kc, m_prev):
        s = _dot(k_v[g, kc * TK:(kc + 1) * TK, :], wq)
        s_ring[slot][...] = s
        cm = jnp.max(jnp.max(s.reshape(TK // 8, 8, TQ), axis=0), axis=0, keepdims=True)
        m = cm if m_prev is None else jnp.maximum(m_prev, cm)
        m_ring[slot][...] = m
        return m

    wq0, g0 = get_wq(0)
    m0 = None
    for t in range(LOOKAHEAD):
        m0 = score_chunk(t % RING, g0, wq0, t, m0)

    def attn_body(i, carry):
        u0 = i * UNITS
        wqs = {}
        ms = {}

        def wq_of(ul):
            if ul not in wqs:
                wqs[ul] = get_wq(jnp.minimum(u0 + ul, NU - 1))
            return wqs[ul]

        def m_of(t):
            if t not in ms:
                ms[t] = m_ring[t % RING][...]
            return ms[t]

        acc = None
        for t in range(STEPS):
            ta = t + LOOKAHEAD
            ul, kc = divmod(ta, NK)
            wq, g = wq_of(ul)
            ms[ta] = score_chunk(ta % RING, g, wq, kc, None if kc == 0 else m_of(ta - 1))
            ul, kc = divmod(t, NK)
            u = u0 + ul
            h = u // NQ
            qi = u % NQ
            hrow = pl.multiple_of(h * HP, HP)
            mt = m_of(t)
            p = jnp.exp2(s_ring[t % RING][...] - mt).astype(_BF16)
            pv = _dot(vt_v[pl.ds(hrow, HP), kc * TK:(kc + 1) * TK], p)
            if kc == 0:
                acc = pv
            else:
                acc = acc * jnp.exp2(m_of(t - 1) - mt) + pv
            if kc == NK - 1:
                qoff = pl.multiple_of(qi * TQ, TQ)
                o = acc / acc[DH:DH + 1, :]
                ot_v[pl.ds(hrow, HP), pl.ds(qoff, TQ)] = o.astype(_BF16)
        return carry

    jax.lax.fori_loop(0, NU // UNITS, attn_body, 0)
    w1_copy.wait()
    b1_copy.wait()
    w2_copy.wait()
    b2_copy.wait()

    for c in range(S // TS3):
        cols = slice(c * TS3, (c + 1) * TS3)
        ht = xt_v[:, cols].astype(_F32) + _dot(wo_t[...], ot_v[:, cols])
        ht_v[:, cols] = ht
        mu = jnp.mean(ht, axis=0, keepdims=True)
        hc = ht - mu
        var = jnp.mean(hc * hc, axis=0, keepdims=True)
        hnt_v[:, cols] = (hc * jax.lax.rsqrt(var + EPS)).astype(_BF16)

    for c in range(F // TF4):
        cols = slice(c * TF4, (c + 1) * TF4)
        u = _dot(hnt_v[...], w1_v[:, cols]) + b1_v[:, cols].astype(_F32)
        g_v[:, cols] = jax.nn.gelu(u, approximate=True).astype(_BF16)

    for c in range(N5):
        cols = slice(c * TS5, (c + 1) * TS5)
        y = _dot(g_v[...], w2_v[:, cols]) + b2_v[:, cols].astype(_F32) + ht_v[:, cols]
        out_v[:, cols] = y.astype(_BF16)
        out_copy(c).start()
    for c in range(N5):
        out_copy(c).wait()


@jax.jit
def pallas_sequential_preLN__mha_block__mixer_token_mlp__prompt_kernel(
    A_x: jax.Array,
    A_wqkv: jax.Array,
    A_wo: jax.Array,
    B_x: jax.Array,
    B_w1: jax.Array,
    B_b1: jax.Array,
    B_w2: jax.Array,
    B_b2: jax.Array,
):
    del B_x
    xt = jnp.transpose(A_x, (0, 2, 1)).reshape(D, S)
    b1 = B_b1.reshape(1, F)
    b2 = B_b2.reshape(1, S)

    scratch = [
        pltpu.VMEM((D, S), _BF16),
        pltpu.VMEM((D, 3 * D), _BF16),
        pltpu.VMEM((D, D), _BF16),
        pltpu.VMEM((S, F), _BF16),
        pltpu.VMEM((1, F), _BF16),
        pltpu.VMEM((F, S), _BF16),
        pltpu.VMEM((1, S), _BF16),
        pltpu.VMEM((2 * D + H * HP, D), _BF16),
        pltpu.VMEM((D, H * HP), _BF16),
        pltpu.VMEM((NG, S, GP), _BF16),
        pltpu.VMEM((NG, GP, S), _BF16),
        pltpu.VMEM((H * HP, S), _BF16),
        pltpu.VMEM((H * HP, S), _BF16),
        pltpu.VMEM((D, S), _F32),
        pltpu.VMEM((D, S), _BF16),
        pltpu.VMEM((D, F), _BF16),
        pltpu.VMEM((D, S), _BF16),
        pltpu.SemaphoreType.DMA((NSEM,)),
    ]
    scratch += [pltpu.VMEM((TK, TQ), _F32)] * RING
    scratch += [pltpu.VMEM((1, TQ), _F32)] * RING

    any_spec = pl.BlockSpec(memory_space=pl.ANY)
    out = pl.pallas_call(
        _kernel,
        out_shape=jax.ShapeDtypeStruct((D, S), _BF16),
        in_specs=[any_spec] * 7,
        out_specs=any_spec,
        scratch_shapes=scratch,
        compiler_params=pltpu.CompilerParams(vmem_limit_bytes=100 * 1024 * 1024),
    )(xt, A_wqkv, A_wo, B_w1, b1, B_w2, b2)
    return jnp.transpose(out.reshape(1, D, S), (0, 2, 1))
```

```python
import functools
import math

import jax
import jax.numpy as jnp
import jax.experimental.pallas as pl
import jax.experimental.pallas.tpu as pltpu

S = 2048
D = 448
H = 16
DH = 28
F = 1792
HPG = 4
NG = H // HPG
GW = HPG * DH
GP = 128
HP = 32
EPS = 1e-5

X_OFFS = (0, 256, 768, 1280, 1792, 2048)
TQ = 1024
TK = 128
LOOKAHEAD = 2
UNITS = 8
TS3 = 512
TF4 = 256
TS5 = 256

NQ = S // TQ
NK = S // TK
NU = H * NQ
STEPS = UNITS * NK
RING = LOOKAHEAD + 1
while STEPS % RING:
    RING += 1

N1 = len(X_OFFS) - 1
X_PIECES = ((0, X_OFFS[1]), (X_OFFS[1], X_OFFS[2]), (X_OFFS[2], S))
W_PIECES = ((0, 512), (512, 2 * D), (2 * D, 3 * D))
N5 = S // TS5

SEM_X = 0
SEM_WQKV = SEM_X + len(X_PIECES)
SEM_WO = SEM_WQKV + len(W_PIECES)
SEM_B1 = SEM_WO + 1
SEM_B2 = SEM_B1 + 1
SEM_W1 = SEM_B2 + 1
SEM_W2 = SEM_W1 + 1
SEM_OUT = SEM_W2 + 1
NSEM = SEM_OUT + N5

_NT = (((1,), (1,)), ((), ()))
_F32 = jnp.float32
_BF16 = jnp.bfloat16


def _dot(a, b):
    return jnp.dot(a, b, preferred_element_type=_F32)


def _dot_nt(a, b):
    return jax.lax.dot_general(a, b, _NT, preferred_element_type=_F32)


def _pad_head_rows(w):
    zeros = jnp.zeros((HP - DH, w.shape[1]), w.dtype)
    parts = []
    for h in range(H):
        parts.append(w[h * DH:(h + 1) * DH, :])
        parts.append(zeros)
    return jnp.concatenate(parts, axis=0)


def _kernel(xt_hbm, wqkv_hbm, wo_hbm, w1_hbm, b1_hbm, w2_hbm, b2_hbm, out_hbm,
            xt_v, wqkv_v, wo_v, w1_v, b1_v, w2_v, b2_v,
            w_t, wo_t, k_v, qt_v, vt_v, ot_v, ht_v, hnt_v, g_v, out_v,
            sems, *ring):
    s_ring = ring[:RING]
    m_ring = ring[RING:]

    def copy(src, dst, sem):
        return pltpu.make_async_copy(src, dst, sems.at[sem])

    def x_copy(i):
        lo, hi = X_PIECES[i]
        cols = pl.ds(lo, hi - lo)
        return copy(xt_hbm.at[:, cols], xt_v.at[:, cols], SEM_X + i)

    def out_copy(c):
        cols = pl.ds(c * TS5, TS5)
        return copy(out_v.at[:, cols], out_hbm.at[:, cols], SEM_OUT + c)

    def w_copy(i):
        lo, hi = W_PIECES[i]
        cols = pl.ds(lo, hi - lo)
        return copy(wqkv_hbm.at[:, cols], wqkv_v.at[:, cols], SEM_WQKV + i)

    wo_copy = copy(wo_hbm, wo_v, SEM_WO)
    b1_copy = copy(b1_hbm, b1_v, SEM_B1)
    b2_copy = copy(b2_hbm, b2_v, SEM_B2)
    w1_copy = copy(w1_hbm, w1_v, SEM_W1)
    w2_copy = copy(w2_hbm, w2_v, SEM_W2)

    x_copy(0).start()
    w_copy(0).start()
    w_copy(1).start()
    w_copy(2).start()
    x_copy(1).start()
    x_copy(2).start()
    wo_copy.start()
    b1_copy.start()
    b2_copy.start()
    w1_copy.start()
    w2_copy.start()
    x_copy(0).wait()
    w_copy(0).wait()

    q_scale = (DH ** -0.5) * math.log2(math.e)

    def ln1(c):
        cols = slice(X_OFFS[c], X_OFFS[c + 1])
        xf = xt_v[:, cols].astype(_F32)
        mu = jnp.mean(xf, axis=0, keepdims=True)
        xc = xf - mu
        var = jnp.mean(xc * xc, axis=0, keepdims=True)
        return (xc * jax.lax.rsqrt(var + EPS)).astype(_BF16)

    def store_q(c, q):
        cols = slice(X_OFFS[c], X_OFFS[c + 1])
        zpad = jnp.zeros((GP - GW, q.shape[1]), _BF16)
        for g in range(NG):
            qg = (q[g * GW:(g + 1) * GW, :] * q_scale).astype(_BF16)
            qt_v[g, :, cols] = jnp.concatenate([qg, zpad], axis=0)

    def store_k(c, k):
        cols = slice(X_OFFS[c], X_OFFS[c + 1])
        zpad = jnp.zeros((GP - GW, k.shape[1]), _BF16)
        for g in range(NG):
            kg = k[g * GW:(g + 1) * GW, :].astype(_BF16)
            k_v[g, cols, :] = jnp.concatenate([kg, zpad], axis=0).T

    def project_qk(c, xn):
        qk = _dot(w_t[0:2 * D, :], xn)
        store_q(c, qk[0:D, :])
        store_k(c, qk[D:2 * D, :])

    def project_v(c, xn):
        cols = slice(X_OFFS[c], X_OFFS[c + 1])
        vt = _dot(w_t[2 * D:, :], xn)
        rid = jax.lax.broadcasted_iota(jnp.int32, vt.shape, 0)
        vt = jnp.where(rid % HP == DH, 1.0, vt)
        vt_v[:, cols] = vt.astype(_BF16)

    (a0, a1), (b0, b1), (c0, c1) = W_PIECES
    w_t[a0:a1, :] = wqkv_v[:, a0:a1].T
    xn = ln1(0)
    w_copy(1).wait()
    w_t[b0:b1, :] = wqkv_v[:, b0:b1].T
    ra = _dot(w_t[a0:a1, :], xn)
    store_q(0, ra[0:D, :])
    w_copy(2).wait()
    wv_t = wqkv_v[:, c0:c1].astype(_F32).T
    w_t[2 * D:, :] = _pad_head_rows(wv_t).astype(_BF16)
    rb = _dot(w_t[b0:b1, :], xn)
    store_k(0, jnp.concatenate([ra[D:, :], rb], axis=0))
    x_copy(1).wait()
    for c in range(1, N1):
        if c == 2:
            x_copy(2).wait()
            wo_copy.wait()
            wo_t[...] = _pad_head_rows(wo_v[...].astype(_F32)).astype(_BF16).T
        xn_next = ln1(c)
        project_v(c - 1, xn)
        project_qk(c, xn_next)
        xn = xn_next
    project_v(N1 - 1, xn)

    def get_wq(u):
        h = u // NQ
        qi = u % NQ
        g = h // HPG
        j = h % HPG
        qoff = pl.multiple_of(qi * TQ, TQ)
        wq = qt_v[g, :, pl.ds(qoff, TQ)]
        rid = jax.lax.broadcasted_iota(jnp.int32, (GP, TQ), 0)
        keep = (rid >= DH * j) & (rid < DH * j + DH)
        return jnp.where(keep, wq, jnp.zeros_like(wq)), g

    def score_chunk(slot, g, wq, kc, m_prev):
        s = _dot(k_v[g, kc * TK:(kc + 1) * TK, :], wq)
        s_ring[slot][...] = s
        cm = jnp.max(jnp.max(s.reshape(TK // 8, 8, TQ), axis=0), axis=0, keepdims=True)
        m = cm if m_prev is None else jnp.maximum(m_prev, cm)
        m_ring[slot][...] = m
        return m

    wq0, g0 = get_wq(0)
    m0 = None
    for t in range(LOOKAHEAD):
        m0 = score_chunk(t % RING, g0, wq0, t, m0)

    def attn_body(i, carry):
        u0 = i * UNITS
        wqs = {}
        ms = {}

        def wq_of(ul):
            if ul not in wqs:
                wqs[ul] = get_wq(jnp.minimum(u0 + ul, NU - 1))
            return wqs[ul]

        def m_of(t):
            if t not in ms:
                ms[t] = m_ring[t % RING][...]
            return ms[t]

        acc = None
        for t in range(STEPS):
            ta = t + LOOKAHEAD
            ul, kc = divmod(ta, NK)
            wq, g = wq_of(ul)
            ms[ta] = score_chunk(ta % RING, g, wq, kc, None if kc == 0 else m_of(ta - 1))
            ul, kc = divmod(t, NK)
            u = u0 + ul
            h = u // NQ
            qi = u % NQ
            hrow = pl.multiple_of(h * HP, HP)
            mt = m_of(t)
            p = jnp.exp2(s_ring[t % RING][...] - mt).astype(_BF16)
            pv = _dot(vt_v[pl.ds(hrow, HP), kc * TK:(kc + 1) * TK], p)
            if kc == 0:
                acc = pv
            else:
                acc = acc * jnp.exp2(m_of(t - 1) - mt) + pv
            if kc == NK - 1:
                qoff = pl.multiple_of(qi * TQ, TQ)
                o = acc / acc[DH:DH + 1, :]
                ot_v[pl.ds(hrow, HP), pl.ds(qoff, TQ)] = o.astype(_BF16)
        return carry

    jax.lax.fori_loop(0, NU // UNITS, attn_body, 0)
    w1_copy.wait()
    b1_copy.wait()
    w2_copy.wait()
    b2_copy.wait()

    for c in range(S // TS3):
        cols = slice(c * TS3, (c + 1) * TS3)
        ht = xt_v[:, cols].astype(_F32) + _dot(wo_t[...], ot_v[:, cols])
        ht_v[:, cols] = ht
        mu = jnp.mean(ht, axis=0, keepdims=True)
        hc = ht - mu
        var = jnp.mean(hc * hc, axis=0, keepdims=True)
        hnt_v[:, cols] = (hc * jax.lax.rsqrt(var + EPS)).astype(_BF16)

    for c in range(F // TF4):
        cols = slice(c * TF4, (c + 1) * TF4)
        u = _dot(hnt_v[...], w1_v[:, cols]) + b1_v[cols].astype(_F32).reshape(1, TF4)
        g_v[:, cols] = jax.nn.gelu(u, approximate=True).astype(_BF16)

    for c in range(N5):
        cols = slice(c * TS5, (c + 1) * TS5)
        y = _dot(g_v[...], w2_v[:, cols]) + b2_v[cols].astype(_F32).reshape(1, TS5) + ht_v[:, cols]
        out_v[:, cols] = y.astype(_BF16)
        out_copy(c).start()
    for c in range(N5):
        out_copy(c).wait()


@jax.jit
def pallas_sequential_preLN__mha_block__mixer_token_mlp__prompt_kernel(
    A_x: jax.Array,
    A_wqkv: jax.Array,
    A_wo: jax.Array,
    B_x: jax.Array,
    B_w1: jax.Array,
    B_b1: jax.Array,
    B_w2: jax.Array,
    B_b2: jax.Array,
):
    del B_x
    xt = jnp.transpose(A_x, (0, 2, 1)).reshape(D, S)

    scratch = [
        pltpu.VMEM((D, S), _BF16),
        pltpu.VMEM((D, 3 * D), _BF16),
        pltpu.VMEM((D, D), _BF16),
        pltpu.VMEM((S, F), _BF16),
        pltpu.VMEM((F,), _BF16),
        pltpu.VMEM((F, S), _BF16),
        pltpu.VMEM((S,), _BF16),
        pltpu.VMEM((2 * D + H * HP, D), _BF16),
        pltpu.VMEM((D, H * HP), _BF16),
        pltpu.VMEM((NG, S, GP), _BF16),
        pltpu.VMEM((NG, GP, S), _BF16),
        pltpu.VMEM((H * HP, S), _BF16),
        pltpu.VMEM((H * HP, S), _BF16),
        pltpu.VMEM((D, S), _F32),
        pltpu.VMEM((D, S), _BF16),
        pltpu.VMEM((D, F), _BF16),
        pltpu.VMEM((D, S), _BF16),
        pltpu.SemaphoreType.DMA((NSEM,)),
    ]
    scratch += [pltpu.VMEM((TK, TQ), _F32)] * RING
    scratch += [pltpu.VMEM((1, TQ), _F32)] * RING

    any_spec = pl.BlockSpec(memory_space=pl.ANY)
    out = pl.pallas_call(
        _kernel,
        out_shape=jax.ShapeDtypeStruct((D, S), _BF16),
        in_specs=[any_spec] * 7,
        out_specs=any_spec,
        scratch_shapes=scratch,
        compiler_params=pltpu.CompilerParams(vmem_limit_bytes=100 * 1024 * 1024),
    )(xt, A_wqkv, A_wo, B_w1, B_b1, B_w2, B_b2)
    return jnp.transpose(out.reshape(1, D, S), (0, 2, 1))
```

```python
import functools
import math

import jax
import jax.numpy as jnp
import jax.experimental.pallas as pl
import jax.experimental.pallas.tpu as pltpu

S = 2048
D = 448
H = 16
DH = 28
F = 1792
HPG = 4
NG = H // HPG
GW = HPG * DH
GP = 128
HP = 32
EPS = 1e-5

X_OFFS = (0, 256, 768, 1280, 1792, 2048)
TQ = 1024
TK = 128
LOOKAHEAD = 2
UNITS = 8
TS3 = 512
TF4 = 256
TS5 = 256

NQ = S // TQ
NK = S // TK
NU = H * NQ
STEPS = UNITS * NK
RING = LOOKAHEAD + 1
while STEPS % RING:
    RING += 1

N1 = len(X_OFFS) - 1
X_PIECES = ((0, X_OFFS[1]), (X_OFFS[1], X_OFFS[2]), (X_OFFS[2], S))
W_PIECES = ((0, 512), (512, 2 * D), (2 * D, 3 * D))
N5 = S // TS5

SEM_X = 0
SEM_WQKV = SEM_X + len(X_PIECES)
SEM_WO = SEM_WQKV + len(W_PIECES)
SEM_B1 = SEM_WO + 1
SEM_B2 = SEM_B1 + 1
SEM_W1 = SEM_B2 + 1
SEM_W2 = SEM_W1 + 1
SEM_OUT = SEM_W2 + 1
NSEM = SEM_OUT + N5

_NT = (((1,), (1,)), ((), ()))
_F32 = jnp.float32
_BF16 = jnp.bfloat16


def _dot(a, b):
    return jnp.dot(a, b, preferred_element_type=_F32)


def _dot_nt(a, b):
    return jax.lax.dot_general(a, b, _NT, preferred_element_type=_F32)


def _pad_head_rows(w):
    zeros = jnp.zeros((HP - DH, w.shape[1]), w.dtype)
    parts = []
    for h in range(H):
        parts.append(w[h * DH:(h + 1) * DH, :])
        parts.append(zeros)
    return jnp.concatenate(parts, axis=0)


def _kernel(xt_hbm, wqkv_hbm, wo_hbm, w1_hbm, b1_hbm, w2_hbm, b2_hbm, out_hbm,
            xt_v, wqkv_v, wo_v, w1_v, b1_v, w2_v, b2_v,
            w_t, wo_t, k_v, qt_v, vt_v, ot_v, ht_v, hnt_v, g_v, out_v,
            sems, *ring):
    s_ring = ring[:RING]
    m_ring = ring[RING:]

    def copy(src, dst, sem):
        return pltpu.make_async_copy(src, dst, sems.at[sem])

    def x_copy(i):
        lo, hi = X_PIECES[i]
        cols = pl.ds(lo, hi - lo)
        return copy(xt_hbm.at[:, cols], xt_v.at[:, cols], SEM_X + i)

    def out_copy(c):
        cols = pl.ds(c * TS5, TS5)
        return copy(out_v.at[:, cols], out_hbm.at[:, cols], SEM_OUT + c)

    def w_copy(i):
        lo, hi = W_PIECES[i]
        cols = pl.ds(lo, hi - lo)
        return copy(wqkv_hbm.at[:, cols], wqkv_v.at[:, cols], SEM_WQKV + i)

    wo_copy = copy(wo_hbm, wo_v, SEM_WO)
    b1_copy = copy(b1_hbm, b1_v, SEM_B1)
    b2_copy = copy(b2_hbm, b2_v, SEM_B2)
    w1_copy = copy(w1_hbm, w1_v, SEM_W1)
    w2_copy = copy(w2_hbm, w2_v, SEM_W2)

    x_copy(0).start()
    w_copy(0).start()
    w_copy(1).start()
    w_copy(2).start()
    x_copy(1).start()
    x_copy(2).start()
    wo_copy.start()
    b1_copy.start()
    b2_copy.start()
    w1_copy.start()
    w2_copy.start()
    x_copy(0).wait()
    w_copy(0).wait()

    q_scale = (DH ** -0.5) * math.log2(math.e)

    def ln1(c):
        cols = slice(X_OFFS[c], X_OFFS[c + 1])
        xf = xt_v[:, cols].astype(_F32)
        mu = jnp.mean(xf, axis=0, keepdims=True)
        xc = xf - mu
        var = jnp.mean(xc * xc, axis=0, keepdims=True)
        return (xc * jax.lax.rsqrt(var + EPS)).astype(_BF16)

    def store_q(c, q):
        cols = slice(X_OFFS[c], X_OFFS[c + 1])
        zpad = jnp.zeros((GP - GW, q.shape[1]), _BF16)
        for g in range(NG):
            qg = (q[g * GW:(g + 1) * GW, :] * q_scale).astype(_BF16)
            qt_v[g, :, cols] = jnp.concatenate([qg, zpad], axis=0)

    def store_k(c, k):
        cols = slice(X_OFFS[c], X_OFFS[c + 1])
        zpad = jnp.zeros((GP - GW, k.shape[1]), _BF16)
        for g in range(NG):
            kg = k[g * GW:(g + 1) * GW, :].astype(_BF16)
            k_v[g, cols, :] = jnp.concatenate([kg, zpad], axis=0).T

    def project_qk(c, xn):
        qk = _dot(w_t[0:2 * D, :], xn)
        store_q(c, qk[0:D, :])
        store_k(c, qk[D:2 * D, :])

    def project_v(c, xn):
        cols = slice(X_OFFS[c], X_OFFS[c + 1])
        vt = _dot(w_t[2 * D:, :], xn)
        tail = (jax.lax.broadcasted_iota(jnp.int32, (HP - DH, vt.shape[1]), 0) == 0).astype(_F32)
        for h in range(H):
            vh = jnp.concatenate([vt[h * DH:(h + 1) * DH, :], tail], axis=0)
            vt_v[h * HP:(h + 1) * HP, cols] = vh.astype(_BF16)

    (a0, a1), (b0, b1), (c0, c1) = W_PIECES
    w_t[a0:a1, :] = wqkv_v[:, a0:a1].T
    xn = ln1(0)
    w_copy(1).wait()
    w_t[b0:b1, :] = wqkv_v[:, b0:b1].T
    ra = _dot(w_t[a0:a1, :], xn)
    store_q(0, ra[0:D, :])
    w_copy(2).wait()
    w_t[c0:c1, :] = wqkv_v[:, c0:c1].T
    rb = _dot(w_t[b0:b1, :], xn)
    store_k(0, jnp.concatenate([ra[D:, :], rb], axis=0))
    x_copy(1).wait()
    for c in range(1, N1):
        if c == 2:
            x_copy(2).wait()
            wo_copy.wait()
            wo_t[...] = _pad_head_rows(wo_v[...].astype(_F32)).astype(_BF16).T
        xn_next = ln1(c)
        project_v(c - 1, xn)
        project_qk(c, xn_next)
        xn = xn_next
    project_v(N1 - 1, xn)

    def get_wq(u):
        h = u // NQ
        qi = u % NQ
        g = h // HPG
        j = h % HPG
        qoff = pl.multiple_of(qi * TQ, TQ)
        wq = qt_v[g, :, pl.ds(qoff, TQ)]
        rid = jax.lax.broadcasted_iota(jnp.int32, (GP, TQ), 0)
        keep = (rid >= DH * j) & (rid < DH * j + DH)
        return jnp.where(keep, wq, jnp.zeros_like(wq)), g

    def score_chunk(slot, g, wq, kc, m_prev):
        s = _dot(k_v[g, kc * TK:(kc + 1) * TK, :], wq)
        s_ring[slot][...] = s
        cm = jnp.max(jnp.max(s.reshape(TK // 8, 8, TQ), axis=0), axis=0, keepdims=True)
        m = cm if m_prev is None else jnp.maximum(m_prev, cm)
        m_ring[slot][...] = m
        return m

    wq0, g0 = get_wq(0)
    m0 = None
    for t in range(LOOKAHEAD):
        m0 = score_chunk(t % RING, g0, wq0, t, m0)

    def attn_body(i, carry):
        u0 = i * UNITS
        wqs = {}
        ms = {}

        def wq_of(ul):
            if ul not in wqs:
                wqs[ul] = get_wq(jnp.minimum(u0 + ul, NU - 1))
            return wqs[ul]

        def m_of(t):
            if t not in ms:
                ms[t] = m_ring[t % RING][...]
            return ms[t]

        acc = None
        for t in range(STEPS):
            ta = t + LOOKAHEAD
            ul, kc = divmod(ta, NK)
            wq, g = wq_of(ul)
            ms[ta] = score_chunk(ta % RING, g, wq, kc, None if kc == 0 else m_of(ta - 1))
            ul, kc = divmod(t, NK)
            u = u0 + ul
            h = u // NQ
            qi = u % NQ
            hrow = pl.multiple_of(h * HP, HP)
            mt = m_of(t)
            p = jnp.exp2(s_ring[t % RING][...] - mt).astype(_BF16)
            pv = _dot(vt_v[pl.ds(hrow, HP), kc * TK:(kc + 1) * TK], p)
            if kc == 0:
                acc = pv
            else:
                acc = acc * jnp.exp2(m_of(t - 1) - mt) + pv
            if kc == NK - 1:
                qoff = pl.multiple_of(qi * TQ, TQ)
                o = acc / acc[DH:DH + 1, :]
                ot_v[pl.ds(hrow, HP), pl.ds(qoff, TQ)] = o.astype(_BF16)
        return carry

    jax.lax.fori_loop(0, NU // UNITS, attn_body, 0)
    w1_copy.wait()
    b1_copy.wait()
    w2_copy.wait()
    b2_copy.wait()

    for c in range(S // TS3):
        cols = slice(c * TS3, (c + 1) * TS3)
        ht = xt_v[:, cols].astype(_F32) + _dot(wo_t[...], ot_v[:, cols])
        ht_v[:, cols] = ht
        mu = jnp.mean(ht, axis=0, keepdims=True)
        hc = ht - mu
        var = jnp.mean(hc * hc, axis=0, keepdims=True)
        hnt_v[:, cols] = (hc * jax.lax.rsqrt(var + EPS)).astype(_BF16)

    for c in range(F // TF4):
        cols = slice(c * TF4, (c + 1) * TF4)
        u = _dot(hnt_v[...], w1_v[:, cols]) + b1_v[cols].astype(_F32).reshape(1, TF4)
        g_v[:, cols] = jax.nn.gelu(u, approximate=True).astype(_BF16)

    for c in range(N5):
        cols = slice(c * TS5, (c + 1) * TS5)
        y = _dot(g_v[...], w2_v[:, cols]) + b2_v[cols].astype(_F32).reshape(1, TS5) + ht_v[:, cols]
        out_v[:, cols] = y.astype(_BF16)
        out_copy(c).start()
    for c in range(N5):
        out_copy(c).wait()


@jax.jit
def pallas_sequential_preLN__mha_block__mixer_token_mlp__prompt_kernel(
    A_x: jax.Array,
    A_wqkv: jax.Array,
    A_wo: jax.Array,
    B_x: jax.Array,
    B_w1: jax.Array,
    B_b1: jax.Array,
    B_w2: jax.Array,
    B_b2: jax.Array,
):
    del B_x
    xt = jnp.transpose(A_x, (0, 2, 1)).reshape(D, S)

    scratch = [
        pltpu.VMEM((D, S), _BF16),
        pltpu.VMEM((D, 3 * D), _BF16),
        pltpu.VMEM((D, D), _BF16),
        pltpu.VMEM((S, F), _BF16),
        pltpu.VMEM((F,), _BF16),
        pltpu.VMEM((F, S), _BF16),
        pltpu.VMEM((S,), _BF16),
        pltpu.VMEM((3 * D, D), _BF16),
        pltpu.VMEM((D, H * HP), _BF16),
        pltpu.VMEM((NG, S, GP), _BF16),
        pltpu.VMEM((NG, GP, S), _BF16),
        pltpu.VMEM((H * HP, S), _BF16),
        pltpu.VMEM((H * HP, S), _BF16),
        pltpu.VMEM((D, S), _F32),
        pltpu.VMEM((D, S), _BF16),
        pltpu.VMEM((D, F), _BF16),
        pltpu.VMEM((D, S), _BF16),
        pltpu.SemaphoreType.DMA((NSEM,)),
    ]
    scratch += [pltpu.VMEM((TK, TQ), _F32)] * RING
    scratch += [pltpu.VMEM((1, TQ), _F32)] * RING

    any_spec = pl.BlockSpec(memory_space=pl.ANY)
    out = pl.pallas_call(
        _kernel,
        out_shape=jax.ShapeDtypeStruct((D, S), _BF16),
        in_specs=[any_spec] * 7,
        out_specs=any_spec,
        scratch_shapes=scratch,
        compiler_params=pltpu.CompilerParams(vmem_limit_bytes=100 * 1024 * 1024),
    )(xt, A_wqkv, A_wo, B_w1, B_b1, B_w2, B_b2)
    return jnp.transpose(out.reshape(1, D, S), (0, 2, 1))
```

```python
import functools
import math

import jax
import jax.numpy as jnp
import jax.experimental.pallas as pl
import jax.experimental.pallas.tpu as pltpu

S = 2048
D = 448
H = 16
DH = 28
F = 1792
HPG = 4
NG = H // HPG
GW = HPG * DH
GP = 128
HP = 32
EPS = 1e-5

X_OFFS = (0, 256, 768, 1280, 1792, 2048)
TQ = 1024
TK = 128
LOOKAHEAD = 2
UNITS = 4
TS3 = 512
TF4 = 256
TS5 = 256

NQ = S // TQ
NK = S // TK
NU = H * NQ
STEPS = UNITS * NK
RING = LOOKAHEAD + 1
while STEPS % RING:
    RING += 1

N1 = len(X_OFFS) - 1
X_PIECES = ((0, X_OFFS[1]), (X_OFFS[1], X_OFFS[2]), (X_OFFS[2], S))
W_PIECES = ((0, 512), (512, 2 * D), (2 * D, 3 * D))
N5 = S // TS5

SEM_X = 0
SEM_WQKV = SEM_X + len(X_PIECES)
SEM_WO = SEM_WQKV + len(W_PIECES)
SEM_B1 = SEM_WO + 1
SEM_B2 = SEM_B1 + 1
SEM_W1 = SEM_B2 + 1
SEM_W2 = SEM_W1 + 1
SEM_OUT = SEM_W2 + 1
NSEM = SEM_OUT + N5

_NT = (((1,), (1,)), ((), ()))
_F32 = jnp.float32
_BF16 = jnp.bfloat16


def _dot(a, b):
    return jnp.dot(a, b, preferred_element_type=_F32)


def _dot_nt(a, b):
    return jax.lax.dot_general(a, b, _NT, preferred_element_type=_F32)


def _pad_head_rows(w):
    zeros = jnp.zeros((HP - DH, w.shape[1]), w.dtype)
    parts = []
    for h in range(H):
        parts.append(w[h * DH:(h + 1) * DH, :])
        parts.append(zeros)
    return jnp.concatenate(parts, axis=0)


def _kernel(xt_hbm, wqkv_hbm, wo_hbm, w1_hbm, b1_hbm, w2_hbm, b2_hbm, out_hbm,
            xt_v, wqkv_v, wo_v, w1_v, b1_v, w2_v, b2_v,
            w_t, wo_t, k_v, qt_v, vt_v, ot_v, ht_v, hnt_v, g_v, out_v,
            sems, *ring):
    s_ring = ring[:RING]
    m_ring = ring[RING:]

    def copy(src, dst, sem):
        return pltpu.make_async_copy(src, dst, sems.at[sem])

    def x_copy(i):
        lo, hi = X_PIECES[i]
        cols = pl.ds(lo, hi - lo)
        return copy(xt_hbm.at[:, cols], xt_v.at[:, cols], SEM_X + i)

    def out_copy(c):
        cols = pl.ds(c * TS5, TS5)
        return copy(out_v.at[:, cols], out_hbm.at[:, cols], SEM_OUT + c)

    def w_copy(i):
        lo, hi = W_PIECES[i]
        cols = pl.ds(lo, hi - lo)
        return copy(wqkv_hbm.at[:, cols], wqkv_v.at[:, cols], SEM_WQKV + i)

    wo_copy = copy(wo_hbm, wo_v, SEM_WO)
    b1_copy = copy(b1_hbm, b1_v, SEM_B1)
    b2_copy = copy(b2_hbm, b2_v, SEM_B2)
    w1_copy = copy(w1_hbm, w1_v, SEM_W1)
    w2_copy = copy(w2_hbm, w2_v, SEM_W2)

    x_copy(0).start()
    w_copy(0).start()
    w_copy(1).start()
    w_copy(2).start()
    x_copy(1).start()
    x_copy(2).start()
    wo_copy.start()
    b1_copy.start()
    b2_copy.start()
    w1_copy.start()
    w2_copy.start()
    x_copy(0).wait()
    w_copy(0).wait()

    q_scale = (DH ** -0.5) * math.log2(math.e)

    def ln1(c):
        cols = slice(X_OFFS[c], X_OFFS[c + 1])
        xf = xt_v[:, cols].astype(_F32)
        mu = jnp.mean(xf, axis=0, keepdims=True)
        xc = xf - mu
        var = jnp.mean(xc * xc, axis=0, keepdims=True)
        return (xc * jax.lax.rsqrt(var + EPS)).astype(_BF16)

    def store_q(c, q):
        cols = slice(X_OFFS[c], X_OFFS[c + 1])
        zpad = jnp.zeros((GP - GW, q.shape[1]), _BF16)
        for g in range(NG):
            qg = (q[g * GW:(g + 1) * GW, :] * q_scale).astype(_BF16)
            qt_v[g, :, cols] = jnp.concatenate([qg, zpad], axis=0)

    def store_k(c, k):
        cols = slice(X_OFFS[c], X_OFFS[c + 1])
        zpad = jnp.zeros((GP - GW, k.shape[1]), _BF16)
        for g in range(NG):
            kg = k[g * GW:(g + 1) * GW, :].astype(_BF16)
            k_v[g, cols, :] = jnp.concatenate([kg, zpad], axis=0).T

    def store_v(c, vt):
        cols = slice(X_OFFS[c], X_OFFS[c + 1])
        tail = (jax.lax.broadcasted_iota(jnp.int32, (HP - DH, vt.shape[1]), 0) == 0).astype(_F32)
        for h in range(H):
            vh = jnp.concatenate([vt[h * DH:(h + 1) * DH, :], tail], axis=0)
            vt_v[h * HP:(h + 1) * HP, cols] = vh.astype(_BF16)

    def proj(lo, hi, xn):
        return _dot(w_t[lo:hi, :], xn)

    (a0, a1), (b0, b1), (c0, c1) = W_PIECES
    w_t[a0:a1, :] = wqkv_v[:, a0:a1].T
    xn = ln1(0)
    r0 = proj(0, 256, xn)
    w_copy(1).wait()
    w_t[b0:b1, :] = wqkv_v[:, b0:b1].T
    r1 = proj(256, a1, xn)
    store_q(0, jnp.concatenate([r0, r1[0:D - 256, :]], axis=0))
    r2 = proj(b0, b0 + 128, xn)
    w_copy(2).wait()
    w_t[c0:c1, :] = wqkv_v[:, c0:c1].T
    r3 = proj(b0 + 128, b1, xn)
    store_k(0, jnp.concatenate([r1[D - 256:, :], r2, r3], axis=0))
    va = proj(c0, c0 + D // 2, xn)
    x_copy(1).wait()
    xn_next = ln1(1)
    vb = proj(c0 + D // 2, c1, xn)
    store_v(0, jnp.concatenate([va, vb], axis=0))
    xn = xn_next
    for c in range(1, N1):
        qk = proj(0, 2 * D, xn)
        if c == 1:
            x_copy(2).wait()
            wo_copy.wait()
            wo_t[...] = _pad_head_rows(wo_v[...].astype(_F32)).astype(_BF16).T
        if c + 1 < N1:
            xn_next = ln1(c + 1)
        vt = proj(c0, c1, xn)
        store_q(c, qk[0:D, :])
        store_k(c, qk[D:2 * D, :])
        store_v(c, vt)
        xn = xn_next

    def get_wq(u):
        h = u // NQ
        qi = u % NQ
        g = h // HPG
        j = h % HPG
        qoff = pl.multiple_of(qi * TQ, TQ)
        wq = qt_v[g, :, pl.ds(qoff, TQ)]
        rid = jax.lax.broadcasted_iota(jnp.int32, (GP, TQ), 0)
        keep = (rid >= DH * j) & (rid < DH * j + DH)
        return jnp.where(keep, wq, jnp.zeros_like(wq)), g

    def score_chunk(slot, g, wq, kc, m_prev):
        s = _dot(k_v[g, kc * TK:(kc + 1) * TK, :], wq)
        s_ring[slot][...] = s
        cm = jnp.max(jnp.max(s.reshape(TK // 8, 8, TQ), axis=0), axis=0, keepdims=True)
        m = cm if m_prev is None else jnp.maximum(m_prev, cm)
        m_ring[slot][...] = m
        return m

    wq0, g0 = get_wq(0)
    m0 = None
    for t in range(LOOKAHEAD):
        m0 = score_chunk(t % RING, g0, wq0, t, m0)

    def attn_body(i, carry):
        u0 = i * UNITS
        wqs = {}
        ms = {}

        def wq_of(ul):
            if ul not in wqs:
                wqs[ul] = get_wq(jnp.minimum(u0 + ul, NU - 1))
            return wqs[ul]

        def m_of(t):
            if t not in ms:
                ms[t] = m_ring[t % RING][...]
            return ms[t]

        acc = None
        for t in range(STEPS):
            ta = t + LOOKAHEAD
            ul, kc = divmod(ta, NK)
            wq, g = wq_of(ul)
            ms[ta] = score_chunk(ta % RING, g, wq, kc, None if kc == 0 else m_of(ta - 1))
            ul, kc = divmod(t, NK)
            u = u0 + ul
            h = u // NQ
            qi = u % NQ
            hrow = pl.multiple_of(h * HP, HP)
            mt = m_of(t)
            p = jnp.exp2(s_ring[t % RING][...] - mt).astype(_BF16)
            pv = _dot(vt_v[pl.ds(hrow, HP), kc * TK:(kc + 1) * TK], p)
            if kc == 0:
                acc = pv
            else:
                acc = acc * jnp.exp2(m_of(t - 1) - mt) + pv
            if kc == NK - 1:
                qoff = pl.multiple_of(qi * TQ, TQ)
                o = acc / acc[DH:DH + 1, :]
                ot_v[pl.ds(hrow, HP), pl.ds(qoff, TQ)] = o.astype(_BF16)
        return carry

    jax.lax.fori_loop(0, NU // UNITS, attn_body, 0)
    w1_copy.wait()
    b1_copy.wait()
    w2_copy.wait()
    b2_copy.wait()

    for c in range(S // TS3):
        cols = slice(c * TS3, (c + 1) * TS3)
        ht = xt_v[:, cols].astype(_F32) + _dot(wo_t[...], ot_v[:, cols])
        ht_v[:, cols] = ht
        mu = jnp.mean(ht, axis=0, keepdims=True)
        hc = ht - mu
        var = jnp.mean(hc * hc, axis=0, keepdims=True)
        hnt_v[:, cols] = (hc * jax.lax.rsqrt(var + EPS)).astype(_BF16)

    for c in range(F // TF4):
        cols = slice(c * TF4, (c + 1) * TF4)
        u = _dot(hnt_v[...], w1_v[:, cols]) + b1_v[cols].astype(_F32).reshape(1, TF4)
        g_v[:, cols] = jax.nn.gelu(u, approximate=True).astype(_BF16)

    for c in range(N5):
        cols = slice(c * TS5, (c + 1) * TS5)
        y = _dot(g_v[...], w2_v[:, cols]) + b2_v[cols].astype(_F32).reshape(1, TS5) + ht_v[:, cols]
        out_v[:, cols] = y.astype(_BF16)
        out_copy(c).start()
    for c in range(N5):
        out_copy(c).wait()


@jax.jit
def pallas_sequential_preLN__mha_block__mixer_token_mlp__prompt_kernel(
    A_x: jax.Array,
    A_wqkv: jax.Array,
    A_wo: jax.Array,
    B_x: jax.Array,
    B_w1: jax.Array,
    B_b1: jax.Array,
    B_w2: jax.Array,
    B_b2: jax.Array,
):
    del B_x
    xt = jnp.transpose(A_x, (0, 2, 1)).reshape(D, S)

    scratch = [
        pltpu.VMEM((D, S), _BF16),
        pltpu.VMEM((D, 3 * D), _BF16),
        pltpu.VMEM((D, D), _BF16),
        pltpu.VMEM((S, F), _BF16),
        pltpu.VMEM((F,), _BF16),
        pltpu.VMEM((F, S), _BF16),
        pltpu.VMEM((S,), _BF16),
        pltpu.VMEM((3 * D, D), _BF16),
        pltpu.VMEM((D, H * HP), _BF16),
        pltpu.VMEM((NG, S, GP), _BF16),
        pltpu.VMEM((NG, GP, S), _BF16),
        pltpu.VMEM((H * HP, S), _BF16),
        pltpu.VMEM((H * HP, S), _BF16),
        pltpu.VMEM((D, S), _F32),
        pltpu.VMEM((D, S), _BF16),
        pltpu.VMEM((D, F), _BF16),
        pltpu.VMEM((D, S), _BF16),
        pltpu.SemaphoreType.DMA((NSEM,)),
    ]
    scratch += [pltpu.VMEM((TK, TQ), _F32)] * RING
    scratch += [pltpu.VMEM((1, TQ), _F32)] * RING

    any_spec = pl.BlockSpec(memory_space=pl.ANY)
    out = pl.pallas_call(
        _kernel,
        out_shape=jax.ShapeDtypeStruct((D, S), _BF16),
        in_specs=[any_spec] * 7,
        out_specs=any_spec,
        scratch_shapes=scratch,
        compiler_params=pltpu.CompilerParams(vmem_limit_bytes=100 * 1024 * 1024),
    )(xt, A_wqkv, A_wo, B_w1, B_b1, B_w2, B_b2)
    return jnp.transpose(out.reshape(1, D, S), (0, 2, 1))
```

```python
import math

import jax
import jax.numpy as jnp
import jax.experimental.pallas as pl
import jax.experimental.pallas.tpu as pltpu

S = 2048
D = 448
H = 16
DH = 28
F = 1792
HPG = 4
NG = H // HPG
GW = HPG * DH
GP = 128
HP = 32
EPS = 1e-5

X_OFFS = (0, 256, 768, 1280, 1792, 2048)
TQ = 1024
TK = 128
LOOKAHEAD = 2
UNITS = 4
TS3 = 128
TF4 = 256
TS5 = 256

NQ = S // TQ
NK = S // TK
NU = H * NQ
assert UNITS % NQ == 0 and HPG == 4
HEADS_PER_BODY = UNITS // NQ
STEPS = UNITS * NK
RING = LOOKAHEAD + 1
while STEPS % RING:
    RING += 1

N1 = len(X_OFFS) - 1
X_PIECES = ((0, X_OFFS[1]), (X_OFFS[1], X_OFFS[2]), (X_OFFS[2], S))
W_PIECES = ((0, 512), (512, 2 * D), (2 * D, 3 * D))
N5 = S // TS5

SEM_X = 0
SEM_WQKV = SEM_X + len(X_PIECES)
SEM_WO = SEM_WQKV + len(W_PIECES)
SEM_B1 = SEM_WO + 1
SEM_B2 = SEM_B1 + 1
SEM_W1 = SEM_B2 + 1
SEM_W2 = SEM_W1 + 1
SEM_OUT = SEM_W2 + 1
NSEM = SEM_OUT + N5

_F32 = jnp.float32
_BF16 = jnp.bfloat16


def _dot(a, b):
    return jnp.dot(a, b, preferred_element_type=_F32)


def _pad_head_rows(w):
    zeros = jnp.zeros((HP - DH, w.shape[1]), w.dtype)
    parts = []
    for h in range(H):
        parts.append(w[h * DH:(h + 1) * DH, :])
        parts.append(zeros)
    return jnp.concatenate(parts, axis=0)


def _kernel(xt_hbm, wqkv_hbm, wo_hbm, w1_hbm, b1_hbm, w2_hbm, b2_hbm, out_hbm,
            xt_v, wqkv_v, wo_v, w1_v, b1_v, w2_v, b2_v,
            w_t, wo_t, k_v, qt_v, vt_v, ot_v, ht_v, hnt_v, g_v, out_v,
            sems, *ring):
    s_ring = ring[:RING]
    m_ring = ring[RING:]

    def copy(src, dst, sem):
        return pltpu.make_async_copy(src, dst, sems.at[sem])

    def x_copy(i):
        lo, hi = X_PIECES[i]
        cols = pl.ds(lo, hi - lo)
        return copy(xt_hbm.at[:, cols], xt_v.at[:, cols], SEM_X + i)

    def out_copy(c):
        cols = pl.ds(c * TS5, TS5)
        return copy(out_v.at[:, cols], out_hbm.at[:, cols], SEM_OUT + c)

    def w_copy(i):
        lo, hi = W_PIECES[i]
        cols = pl.ds(lo, hi - lo)
        return copy(wqkv_hbm.at[:, cols], wqkv_v.at[:, cols], SEM_WQKV + i)

    wo_copy = copy(wo_hbm, wo_v, SEM_WO)
    b1_copy = copy(b1_hbm, b1_v, SEM_B1)
    b2_copy = copy(b2_hbm, b2_v, SEM_B2)
    w1_copy = copy(w1_hbm, w1_v, SEM_W1)
    w2_copy = copy(w2_hbm, w2_v, SEM_W2)

    x_copy(0).start()
    w_copy(0).start()
    w_copy(1).start()
    w_copy(2).start()
    x_copy(1).start()
    x_copy(2).start()
    wo_copy.start()
    b1_copy.start()
    b2_copy.start()
    w1_copy.start()
    w2_copy.start()
    x_copy(0).wait()
    w_copy(0).wait()

    q_scale = (DH ** -0.5) * math.log2(math.e)

    def ln1(c):
        cols = slice(X_OFFS[c], X_OFFS[c + 1])
        xf = xt_v[:, cols].astype(_F32)
        mu = jnp.mean(xf, axis=0, keepdims=True)
        xc = xf - mu
        var = jnp.mean(xc * xc, axis=0, keepdims=True)
        return (xc * jax.lax.rsqrt(var + EPS)).astype(_BF16)

    def store_q(c, q):
        cols = slice(X_OFFS[c], X_OFFS[c + 1])
        zpad = jnp.zeros((GP - GW, q.shape[1]), _BF16)
        for g in range(NG):
            qg = (q[g * GW:(g + 1) * GW, :] * q_scale).astype(_BF16)
            qt_v[g, :, cols] = jnp.concatenate([qg, zpad], axis=0)

    def store_k(c, k):
        cols = slice(X_OFFS[c], X_OFFS[c + 1])
        zpad = jnp.zeros((GP - GW, k.shape[1]), _BF16)
        for g in range(NG):
            kg = k[g * GW:(g + 1) * GW, :].astype(_BF16)
            k_v[g, cols, :] = jnp.concatenate([kg, zpad], axis=0).T

    def store_v(c, vt):
        cols = slice(X_OFFS[c], X_OFFS[c + 1])
        tail = (jax.lax.broadcasted_iota(jnp.int32, (HP - DH, vt.shape[1]), 0) == 0).astype(_F32)
        for h in range(H):
            vh = jnp.concatenate([vt[h * DH:(h + 1) * DH, :], tail], axis=0)
            vt_v[h * HP:(h + 1) * HP, cols] = vh.astype(_BF16)

    def proj(lo, hi, xn):
        return _dot(w_t[lo:hi, :], xn)

    (a0, a1), (b0, b1), (c0, c1) = W_PIECES
    w_t[a0:a1, :] = wqkv_v[:, a0:a1].T
    xn = ln1(0)
    r0 = proj(0, 256, xn)
    w_copy(1).wait()
    w_t[b0:b1, :] = wqkv_v[:, b0:b1].T
    r1 = proj(256, a1, xn)
    store_q(0, jnp.concatenate([r0, r1[0:D - 256, :]], axis=0))
    r2 = proj(b0, b0 + 128, xn)
    w_copy(2).wait()
    w_t[c0:c1, :] = wqkv_v[:, c0:c1].T
    r3 = proj(b0 + 128, b1, xn)
    store_k(0, jnp.concatenate([r1[D - 256:, :], r2, r3], axis=0))
    va = proj(c0, c0 + D // 2, xn)
    x_copy(1).wait()
    xn_next = ln1(1)
    vb = proj(c0 + D // 2, c1, xn)
    store_v(0, jnp.concatenate([va, vb], axis=0))
    xn = xn_next
    for c in range(1, N1):
        qk = proj(0, 2 * D, xn)
        if c == 1:
            x_copy(2).wait()
            wo_copy.wait()
            wo_t[...] = _pad_head_rows(wo_v[...].astype(_F32)).astype(_BF16).T
        if c + 1 < N1:
            xn_next = ln1(c + 1)
        vt = proj(c0, c1, xn)
        store_q(c, qk[0:D, :])
        store_k(c, qk[D:2 * D, :])
        store_v(c, vt)
        xn = xn_next

    def get_wq(h, qi):
        g = jax.lax.shift_right_logical(h, jnp.int32(2))
        j = jax.lax.bitwise_and(h, jnp.int32(HPG - 1))
        wq = qt_v[g, :, qi * TQ:(qi + 1) * TQ]
        rid = jax.lax.broadcasted_iota(jnp.int32, (GP, TQ), 0)
        keep = (rid >= DH * j) & (rid < DH * j + DH)
        return jnp.where(keep, wq, jnp.zeros_like(wq)), g

    def score_chunk(slot, g, wq, kc, m_prev, keep_m):
        s = _dot(k_v[g, kc * TK:(kc + 1) * TK, :], wq)
        s_ring[slot][...] = s
        cm = jnp.max(jnp.max(s.reshape(TK // 8, 8, TQ), axis=0), axis=0, keepdims=True)
        m = cm if m_prev is None else jnp.maximum(m_prev, cm)
        if keep_m:
            m_ring[slot][...] = jnp.broadcast_to(m, (8, TQ))
        return m

    wq0, g0 = get_wq(jnp.int32(0), 0)
    m0 = None
    for t in range(LOOKAHEAD):
        m0 = score_chunk(t % RING, g0, wq0, t, m0, True)

    def attn_body(i, carry):
        h0 = i * HEADS_PER_BODY
        wqs = {}
        ms = {}

        def wq_of(ul):
            if ul not in wqs:
                wqs[ul] = get_wq(jnp.minimum(h0 + ul // NQ, H - 1), ul % NQ)
            return wqs[ul]

        def m_of(t):
            if t not in ms:
                ms[t] = m_ring[t % RING][0:1, :]
            return ms[t]

        acc = None
        for t in range(STEPS):
            ta = t + LOOKAHEAD
            ul, kc = divmod(ta, NK)
            wq, g = wq_of(ul)
            ms[ta] = score_chunk(ta % RING, g, wq, kc,
                                 None if kc == 0 else m_of(ta - 1), ta >= STEPS)
            ul, kc = divmod(t, NK)
            qi = ul % NQ
            hrow = pl.multiple_of((h0 + ul // NQ) * HP, HP)
            mt = m_of(t)
            p = jnp.exp2(s_ring[t % RING][...] - mt).astype(_BF16)
            pv = _dot(vt_v[pl.ds(hrow, HP), kc * TK:(kc + 1) * TK], p)
            if kc == 0:
                acc = pv
            else:
                acc = acc * jnp.exp2(m_of(t - 1) - mt) + pv
            if kc == NK - 1:
                o = acc / acc[DH:DH + 1, :]
                ot_v[pl.ds(hrow, HP), qi * TQ:(qi + 1) * TQ] = o.astype(_BF16)
        return carry

    jax.lax.fori_loop(0, NU // UNITS, attn_body, 0)
    w1_copy.wait()
    b1_copy.wait()
    w2_copy.wait()
    b2_copy.wait()

    for c in range(S // TS3):
        cols = slice(c * TS3, (c + 1) * TS3)
        ht = xt_v[:, cols].astype(_F32) + _dot(wo_t[...], ot_v[:, cols])
        ht_v[:, cols] = ht
        mu = jnp.mean(ht, axis=0, keepdims=True)
        hc = ht - mu
        var = jnp.mean(hc * hc, axis=0, keepdims=True)
        hnt_v[:, cols] = (hc * jax.lax.rsqrt(var + EPS)).astype(_BF16)

    for c in range(F // TF4):
        cols = slice(c * TF4, (c + 1) * TF4)
        u = _dot(hnt_v[...], w1_v[:, cols]) + b1_v[cols].astype(_F32).reshape(1, TF4)
        g_v[:, cols] = jax.nn.gelu(u, approximate=True).astype(_BF16)

    for c in range(N5):
        cols = slice(c * TS5, (c + 1) * TS5)
        y = _dot(g_v[...], w2_v[:, cols]) + b2_v[cols].astype(_F32).reshape(1, TS5) + ht_v[:, cols]
        out_v[:, cols] = y.astype(_BF16)
        out_copy(c).start()
    for c in range(N5):
        out_copy(c).wait()


@jax.jit
def pallas_sequential_preLN__mha_block__mixer_token_mlp__prompt_kernel(
    A_x: jax.Array,
    A_wqkv: jax.Array,
    A_wo: jax.Array,
    B_x: jax.Array,
    B_w1: jax.Array,
    B_b1: jax.Array,
    B_w2: jax.Array,
    B_b2: jax.Array,
):
    del B_x
    xt = jnp.transpose(A_x, (0, 2, 1)).reshape(D, S)

    scratch = [
        pltpu.VMEM((D, S), _BF16),
        pltpu.VMEM((D, 3 * D), _BF16),
        pltpu.VMEM((D, D), _BF16),
        pltpu.VMEM((S, F), _BF16),
        pltpu.VMEM((F,), _BF16),
        pltpu.VMEM((F, S), _BF16),
        pltpu.VMEM((S,), _BF16),
        pltpu.VMEM((3 * D, D), _BF16),
        pltpu.VMEM((D, H * HP), _BF16),
        pltpu.VMEM((NG, S, GP), _BF16),
        pltpu.VMEM((NG, GP, S), _BF16),
        pltpu.VMEM((H * HP, S), _BF16),
        pltpu.VMEM((H * HP, S), _BF16),
        pltpu.VMEM((D, S), _F32),
        pltpu.VMEM((D, S), _BF16),
        pltpu.VMEM((D, F), _BF16),
        pltpu.VMEM((D, S), _BF16),
        pltpu.SemaphoreType.DMA((NSEM,)),
    ]
    scratch += [pltpu.VMEM((TK, TQ), _F32)] * RING
    scratch += [pltpu.VMEM((8, TQ), _F32)] * RING

    any_spec = pl.BlockSpec(memory_space=pl.ANY)
    out = pl.pallas_call(
        _kernel,
        out_shape=jax.ShapeDtypeStruct((D, S), _BF16),
        in_specs=[any_spec] * 7,
        out_specs=any_spec,
        scratch_shapes=scratch,
        compiler_params=pltpu.CompilerParams(vmem_limit_bytes=100 * 1024 * 1024),
    )(xt, A_wqkv, A_wo, B_w1, B_b1, B_w2, B_b2)
    return jnp.transpose(out.reshape(1, D, S), (0, 2, 1))
```

```python
import math

import jax
import jax.numpy as jnp
import jax.experimental.pallas as pl
import jax.experimental.pallas.tpu as pltpu

S = 2048
D = 448
H = 16
DH = 28
F = 1792
HPG = 4
NG = H // HPG
GW = HPG * DH
GP = 128
HP = 32
EPS = 1e-5

X_OFFS = (0, 256, 768, 1280, 1792, 2048)
TQ = 1024
TK = 128
LOOKAHEAD = 2
UNITS = 4
TS3 = 128
TF4 = 256
TS5 = 256

NQ = S // TQ
NK = S // TK
NU = H * NQ
assert UNITS % NQ == 0 and HPG == 4
HEADS_PER_BODY = UNITS // NQ
STEPS = UNITS * NK
RING = LOOKAHEAD + 1
while STEPS % RING:
    RING += 1

N1 = len(X_OFFS) - 1
X_PIECES = ((0, X_OFFS[1]), (X_OFFS[1], X_OFFS[2]), (X_OFFS[2], S))
W_PIECES = ((0, 512), (512, 2 * D), (2 * D, 3 * D))
N5 = S // TS5

SEM_X = 0
SEM_WQKV = SEM_X + len(X_PIECES)
SEM_WO = SEM_WQKV + len(W_PIECES)
SEM_B1 = SEM_WO + 1
SEM_B2 = SEM_B1 + 1
SEM_W1 = SEM_B2 + 1
SEM_W2 = SEM_W1 + 1
SEM_OUT = SEM_W2 + 1
NSEM = SEM_OUT + N5

_F32 = jnp.float32
_BF16 = jnp.bfloat16


def _dot(a, b):
    return jnp.dot(a, b, preferred_element_type=_F32)


def _pad_head_rows(w):
    zeros = jnp.zeros((HP - DH, w.shape[1]), w.dtype)
    parts = []
    for h in range(H):
        parts.append(w[h * DH:(h + 1) * DH, :])
        parts.append(zeros)
    return jnp.concatenate(parts, axis=0)


def _kernel(xt_hbm, wqkv_hbm, wo_hbm, w1_hbm, b1_hbm, w2_hbm, b2_hbm, out_hbm,
            xt_v, wqkv_v, wo_v, w1_v, b1_v, w2_v, b2_v,
            w_t, wo_t, k_v, qt_v, vt_v, ot_v, ht_v, hnt_v, g_v, out_v,
            sems, *ring):
    s_ring = ring[:RING]
    m_ring = ring[RING:]

    def copy(src, dst, sem):
        return pltpu.make_async_copy(src, dst, sems.at[sem])

    def x_copy(i):
        lo, hi = X_PIECES[i]
        cols = pl.ds(lo, hi - lo)
        return copy(xt_hbm.at[:, cols], xt_v.at[:, cols], SEM_X + i)

    def out_copy(c):
        cols = pl.ds(c * TS5, TS5)
        return copy(out_v.at[:, cols], out_hbm.at[:, cols], SEM_OUT + c)

    def w_copy(i):
        lo, hi = W_PIECES[i]
        cols = pl.ds(lo, hi - lo)
        return copy(wqkv_hbm.at[:, cols], wqkv_v.at[:, cols], SEM_WQKV + i)

    wo_copy = copy(wo_hbm, wo_v, SEM_WO)
    b1_copy = copy(b1_hbm, b1_v, SEM_B1)
    b2_copy = copy(b2_hbm, b2_v, SEM_B2)
    w1_copy = copy(w1_hbm, w1_v, SEM_W1)
    w2_copy = copy(w2_hbm, w2_v, SEM_W2)

    x_copy(0).start()
    w_copy(0).start()
    w_copy(1).start()
    w_copy(2).start()
    x_copy(1).start()
    x_copy(2).start()
    wo_copy.start()
    b1_copy.start()
    b2_copy.start()
    w1_copy.start()
    w2_copy.start()
    x_copy(0).wait()
    w_copy(0).wait()

    q_scale = (DH ** -0.5) * math.log2(math.e)

    def ln1(c):
        cols = slice(X_OFFS[c], X_OFFS[c + 1])
        xf = xt_v[:, cols].astype(_F32)
        mu = jnp.mean(xf, axis=0, keepdims=True)
        xc = xf - mu
        var = jnp.mean(xc * xc, axis=0, keepdims=True)
        return (xc * jax.lax.rsqrt(var + EPS)).astype(_BF16)

    def store_q(c, q):
        cols = slice(X_OFFS[c], X_OFFS[c + 1])
        zpad = jnp.zeros((GP - GW, q.shape[1]), _BF16)
        for g in range(NG):
            qg = (q[g * GW:(g + 1) * GW, :] * q_scale).astype(_BF16)
            qt_v[g, :, cols] = jnp.concatenate([qg, zpad], axis=0)

    def store_k(c, k):
        cols = slice(X_OFFS[c], X_OFFS[c + 1])
        zpad = jnp.zeros((GP - GW, k.shape[1]), _BF16)
        for g in range(NG):
            kg = k[g * GW:(g + 1) * GW, :].astype(_BF16)
            k_v[g, cols, :] = jnp.concatenate([kg, zpad], axis=0).T

    def store_v(c, vt):
        cols = slice(X_OFFS[c], X_OFFS[c + 1])
        tail = (jax.lax.broadcasted_iota(jnp.int32, (HP - DH, vt.shape[1]), 0) == 0).astype(_F32)
        for h in range(H):
            vh = jnp.concatenate([vt[h * DH:(h + 1) * DH, :], tail], axis=0)
            vt_v[h * HP:(h + 1) * HP, cols] = vh.astype(_BF16)

    def proj(lo, hi, xn):
        return _dot(w_t[lo:hi, :], xn)

    (a0, a1), (b0, b1), (c0, c1) = W_PIECES
    w_t[a0:a1, :] = wqkv_v[:, a0:a1].T
    xn = ln1(0)
    r0 = proj(0, 256, xn)
    w_copy(1).wait()
    w_t[b0:b1, :] = wqkv_v[:, b0:b1].T
    r1 = proj(256, a1, xn)
    store_q(0, jnp.concatenate([r0, r1[0:D - 256, :]], axis=0))
    r2 = proj(b0, b0 + 128, xn)
    w_copy(2).wait()
    w_t[c0:c1, :] = wqkv_v[:, c0:c1].T
    r3 = proj(b0 + 128, b1, xn)
    store_k(0, jnp.concatenate([r1[D - 256:, :], r2, r3], axis=0))
    va = proj(c0, c0 + D // 2, xn)
    x_copy(1).wait()
    xn_next = ln1(1)
    vb = proj(c0 + D // 2, c1, xn)
    store_v(0, jnp.concatenate([va, vb], axis=0))
    xn = xn_next
    for c in range(1, N1):
        qk = proj(0, 2 * D, xn)
        if c == 1:
            x_copy(2).wait()
            wo_copy.wait()
            wo_t[...] = _pad_head_rows(wo_v[...].astype(_F32)).astype(_BF16).T
        if c + 1 < N1:
            xn_next = ln1(c + 1)
        vt = proj(c0, c1, xn)
        store_q(c, qk[0:D, :])
        store_k(c, qk[D:2 * D, :])
        store_v(c, vt)
        xn = xn_next

    def get_wq(h, qi):
        g = jax.lax.shift_right_logical(h, jnp.int32(2))
        j = jax.lax.bitwise_and(h, jnp.int32(HPG - 1))
        wq = qt_v[g, :, qi * TQ:(qi + 1) * TQ]
        rid = jax.lax.broadcasted_iota(jnp.int32, (GP, TQ), 0)
        keep = (rid >= DH * j) & (rid < DH * j + DH)
        return jnp.where(keep, wq, jnp.zeros_like(wq)), g

    def score_chunk(slot, g, wq, kc, m_prev):
        s = _dot(k_v[g, kc * TK:(kc + 1) * TK, :], wq)
        s_ring[slot][...] = s
        cm = jnp.max(jnp.max(s.reshape(TK // 8, 8, TQ), axis=0), axis=0, keepdims=True)
        m = cm if m_prev is None else jnp.maximum(m_prev, cm)
        m_ring[slot][...] = m
        return m

    wq0, g0 = get_wq(jnp.int32(0), 0)
    m0 = None
    for t in range(LOOKAHEAD):
        m0 = score_chunk(t % RING, g0, wq0, t, m0)

    def attn_body(i, carry):
        h0 = i * HEADS_PER_BODY
        wqs = {}
        ms = {}

        def wq_of(ul):
            if ul not in wqs:
                wqs[ul] = get_wq(jnp.minimum(h0 + ul // NQ, H - 1), ul % NQ)
            return wqs[ul]

        def m_of(t):
            if t not in ms:
                ms[t] = m_ring[t % RING][...]
            return ms[t]

        acc = None
        for t in range(STEPS):
            ta = t + LOOKAHEAD
            ul, kc = divmod(ta, NK)
            wq, g = wq_of(ul)
            ms[ta] = score_chunk(ta % RING, g, wq, kc, None if kc == 0 else m_of(ta - 1))
            ul, kc = divmod(t, NK)
            qi = ul % NQ
            hrow = pl.multiple_of((h0 + ul // NQ) * HP, HP)
            mt = m_of(t)
            p = jnp.exp2(s_ring[t % RING][...] - mt).astype(_BF16)
            pv = _dot(vt_v[pl.ds(hrow, HP), kc * TK:(kc + 1) * TK], p)
            if kc == 0:
                acc = pv
            else:
                acc = acc * jnp.exp2(m_of(t - 1) - mt) + pv
            if kc == NK - 1:
                o = acc / acc[DH:DH + 1, :]
                ot_v[pl.ds(hrow, HP), qi * TQ:(qi + 1) * TQ] = o.astype(_BF16)
        return carry

    jax.lax.fori_loop(0, NU // UNITS, attn_body, 0)
    w1_copy.wait()
    b1_copy.wait()
    w2_copy.wait()
    b2_copy.wait()

    for c in range(S // TS3):
        cols = slice(c * TS3, (c + 1) * TS3)
        ht = xt_v[:, cols].astype(_F32) + _dot(wo_t[...], ot_v[:, cols])
        ht_v[:, cols] = ht
        mu = jnp.mean(ht, axis=0, keepdims=True)
        hc = ht - mu
        var = jnp.mean(hc * hc, axis=0, keepdims=True)
        hnt_v[:, cols] = (hc * jax.lax.rsqrt(var + EPS)).astype(_BF16)

    for c in range(F // TF4):
        cols = slice(c * TF4, (c + 1) * TF4)
        u = _dot(hnt_v[...], w1_v[:, cols]) + b1_v[cols].astype(_F32).reshape(1, TF4)
        g_v[:, cols] = jax.nn.gelu(u, approximate=True).astype(_BF16)

    for c in range(N5):
        cols = slice(c * TS5, (c + 1) * TS5)
        y = _dot(g_v[...], w2_v[:, cols]) + b2_v[cols].astype(_F32).reshape(1, TS5) + ht_v[:, cols]
        out_v[:, cols] = y.astype(_BF16)
        out_copy(c).start()
    for c in range(N5):
        out_copy(c).wait()


@jax.jit
def pallas_sequential_preLN__mha_block__mixer_token_mlp__prompt_kernel(
    A_x: jax.Array,
    A_wqkv: jax.Array,
    A_wo: jax.Array,
    B_x: jax.Array,
    B_w1: jax.Array,
    B_b1: jax.Array,
    B_w2: jax.Array,
    B_b2: jax.Array,
):
    del B_x
    xt = jnp.transpose(A_x, (0, 2, 1)).reshape(D, S)

    scratch = [
        pltpu.VMEM((D, S), _BF16),
        pltpu.VMEM((D, 3 * D), _BF16),
        pltpu.VMEM((D, D), _BF16),
        pltpu.VMEM((S, F), _BF16),
        pltpu.VMEM((F,), _BF16),
        pltpu.VMEM((F, S), _BF16),
        pltpu.VMEM((S,), _BF16),
        pltpu.VMEM((3 * D, D), _BF16),
        pltpu.VMEM((D, H * HP), _BF16),
        pltpu.VMEM((NG, S, GP), _BF16),
        pltpu.VMEM((NG, GP, S), _BF16),
        pltpu.VMEM((H * HP, S), _BF16),
        pltpu.VMEM((H * HP, S), _BF16),
        pltpu.VMEM((D, S), _F32),
        pltpu.VMEM((D, S), _BF16),
        pltpu.VMEM((D, F), _BF16),
        pltpu.VMEM((D, S), _BF16),
        pltpu.SemaphoreType.DMA((NSEM,)),
    ]
    scratch += [pltpu.VMEM((TK, TQ), _F32)] * RING
    scratch += [pltpu.VMEM((1, TQ), _F32)] * RING

    any_spec = pl.BlockSpec(memory_space=pl.ANY)
    out = pl.pallas_call(
        _kernel,
        out_shape=jax.ShapeDtypeStruct((D, S), _BF16),
        in_specs=[any_spec] * 7,
        out_specs=any_spec,
        scratch_shapes=scratch,
        compiler_params=pltpu.CompilerParams(vmem_limit_bytes=100 * 1024 * 1024),
    )(xt, A_wqkv, A_wo, B_w1, B_b1, B_w2, B_b2)
    return jnp.transpose(out.reshape(1, D, S), (0, 2, 1))
```
